```python
import jax
import jax.numpy as jnp

def _softmax(x, axis=-1):
    return jax.nn.softmax(x, axis=axis)

def _gelu(x):
    return jax.nn.gelu(x, approximate=True)

def _silu(x):
    return jax.nn.silu(x)

def _sigmoid(x):
    return jax.nn.sigmoid(x)

def _layernorm(x, axis=-1, eps=1e-05):
    m = jnp.mean(x, axis=axis, keepdims=True)
    v = jnp.var(x, axis=axis, keepdims=True)
    return (x - m) / jnp.sqrt(v + eps)

def _scatter_add(tgt, idx, src, axis=0):
    return tgt.at[idx].add(src)

def _segment_sum(src, seg, n):
    return jax.ops.segment_sum(src, seg, n)

class _Rng:

    def __init__(self, key):
        self._k = key

    def _next(self):
        self._k, sub = jax.random.split(self._k)
        return sub

    def normal(self, shape):
        return jax.random.normal(self._next(), shape, dtype=jnp.bfloat16)

    def randint(self, lo, hi, shape):
        return jax.random.randint(self._next(), shape, lo, hi, dtype=jnp.int32)

    def uniform(self, shape, lo=0.0, hi=1.0):
        return jax.random.uniform(self._next(), shape, jnp.bfloat16, lo, hi)

    def permutation(self, n):
        return jax.random.permutation(self._next(), n)
kernel_name = 'interleave_layers__memory_aug_recurrent_mem_tr__ssm_conv_h3__prompt'

def setup_inputs():
    _rng = _Rng(jax.random.key(int.from_bytes(__import__("os").urandom(4), "little")))
    _w = lambda a: (lambda t: t.astype(jnp.bfloat16) if jnp.issubdtype(t.dtype, jnp.floating) else t)(jnp.asarray(a))

    def _A_setup():
        B, S, Dm = (1, 2048, 640)
        H, Dh = (32, 128)
        M, seg = (8, 32)
        seg = min(seg, S)
        S = S // seg * seg
        return {'x': _w((lambda *s: _rng.normal(s) * 0.05)(B, S, Dm)), 'mem0': _w((lambda *s: _rng.normal(s) * 0.05)(B, M, Dm)), 'Wq': _w((lambda *s: _rng.normal(s) * 0.05)(Dm, H, Dh) * Dm ** (-0.5)), 'Wk': _w((lambda *s: _rng.normal(s) * 0.05)(Dm, H, Dh) * Dm ** (-0.5)), 'Wv': _w((lambda *s: _rng.normal(s) * 0.05)(Dm, H, Dh) * Dm ** (-0.5)), 'Wo': _w((lambda *s: _rng.normal(s) * 0.05)(H, Dh, Dm) * (H * Dh) ** (-0.5)), 'seg_len': seg}
    _A_in = _A_setup()

    def _B_setup():
        B, S, D = (1, 2048, 640)
        ks = 4
        return {'q': _w((lambda *s: _rng.normal(s) * 0.05)(B, S, D)), 'k': _w((lambda *s: _rng.normal(s) * 0.05)(B, S, D)), 'v': _w((lambda *s: _rng.normal(s) * 0.05)(B, S, D)), 'shift_k': _w((lambda *s: _rng.normal(s) * 0.05)(D, ks) * 0.5), 'ssm_k': _w((lambda *s: _rng.normal(s) * 0.05)(D, S) * (1.0 / S ** 0.5)), 'ssm_D': _w((lambda *s: _rng.normal(s) * 0.05)(D))}
    _B_in = _B_setup()
    return {'A_x': _A_in['x'], 'A_mem0': _A_in['mem0'], 'A_Wq': _A_in['Wq'], 'A_Wk': _A_in['Wk'], 'A_Wv': _A_in['Wv'], 'A_Wo': _A_in['Wo'], 'A_seg_len': _A_in['seg_len'], 'B_q': _B_in['q'], 'B_k': _B_in['k'], 'B_v': _B_in['v'], 'B_shift_k': _B_in['shift_k'], 'B_ssm_k': _B_in['ssm_k'], 'B_ssm_D': _B_in['ssm_D']}

def reference(A_x, A_mem0, A_Wq, A_Wk, A_Wv, A_Wo, A_seg_len, B_q, B_k, B_v, B_shift_k, B_ssm_k, B_ssm_D):

    def _A_ref(x, mem0, Wq, Wk, Wv, Wo, seg_len):
        B, S, Dm = x.shape
        H, Dh = (Wq.shape[1], Wq.shape[2])
        M = mem0.shape[1]
        scale = Dh ** (-0.5)
        n_seg = S // seg_len
        L = M + seg_len
        idx = jnp.arange(L)
        mask = (idx[:, None] < M) | (idx[:, None] >= idx[None, :])
        mem = mem0
        outs = []
        for s in range(n_seg):
            xs = x[:, s * seg_len:(s + 1) * seg_len, :].copy()
            h = jnp.concatenate([mem, xs], axis=1)
            q = jnp.einsum('btd,dhe->bhte', h, Wq)
            k = jnp.einsum('btd,dhe->bhte', h, Wk)
            v = jnp.einsum('btd,dhe->bhte', h, Wv)
            scores = jnp.einsum('bhqe,bhke->bhqk', q, k) * scale
            scores = jnp.where(mask[None, None], scores, -1000000000.0)
            p = _softmax(scores, axis=-1)
            o = jnp.einsum('bhqk,bhke->bhqe', p, v)
            o = jnp.einsum('bhte,hed->btd', o, Wo)
            mem = o[:, :M, :].copy()
            outs.append(o[:, M:, :])
        return jnp.concatenate(outs, axis=1)

    def _B_ref(q, k, v, shift_k, ssm_k, ssm_D):
        B, S, D = q.shape
        ks = shift_k.shape[-1]
        k_pad = jnp.pad(k, ((0, 0), (ks - 1, 0), (0, 0)))
        k_shift = jnp.zeros_like(k)
        for t in range(ks):
            k_shift = k_shift + k_pad[:, t:t + S, :] * shift_k[:, ks - 1 - t][None, None, :]
        kv = k_shift * v
        L = 2 * S
        kv_pad = jnp.pad(kv, ((0, 0), (0, S), (0, 0)))
        kf_pad = jnp.pad(ssm_k, ((0, 0), (0, S)))
        kv_f = (lambda x, axes=(-2, -1): jnp.fft.rfft2(x.astype(jnp.float32), axes=axes))(kv_pad[:, None, :, :], axes=(1, 2))
        kf_f = (lambda x, axes=(-2, -1): jnp.fft.rfft2(x.astype(jnp.float32), axes=axes))(kf_pad[:, None, :], axes=(1, 2))
        kf_f = (lambda x, *d: x.transpose(*d))(kf_f, 1, 2, 0)
        y_f = kv_f * kf_f[None, :, :, :]
        y = (lambda x, s, axes=(-2, -1): jnp.fft.irfft2(x, s=s, axes=axes).astype(jnp.bfloat16))(y_f, (1, L), axes=(1, 2))[:, 0, :S, :]
        y = y + kv * ssm_D[None, None, :]
        return q * y
    x = A_x
    x = x + _A_ref(_layernorm(x, axis=-1), A_mem0, A_Wq, A_Wk, A_Wv, A_Wo, A_seg_len)
    x = x + _B_ref(_layernorm(x, axis=-1), B_k, B_v, B_shift_k, B_ssm_k, B_ssm_D)
    x = x + _A_ref(_layernorm(x, axis=-1), A_mem0, A_Wq, A_Wk, A_Wv, A_Wo, A_seg_len)
    x = x + _B_ref(_layernorm(x, axis=-1), B_k, B_v, B_shift_k, B_ssm_k, B_ssm_D)
    return x
```

```python
import functools
import numpy as np
import jax
import jax.numpy as jnp
from jax import lax
from jax.experimental import pallas as pl
from jax.experimental.pallas import tpu as pltpu

S, D, H, DH, M, SEG = 2048, 640, 32, 128, 8, 32
NSEG = S // SEG
R = 2 * (M + SEG)
C = 128
NCH = S // C
NCT = D // 128
F32, BF16 = jnp.float32, jnp.bfloat16
LAGPV = 2
EPS = 1e-5


def _consts():
    N = 2 * C
    f = np.arange(C)[:, None].astype(np.float64)
    t = np.arange(N)[None, :].astype(np.float64)
    th = np.pi * (2 * f + 1) * t / N
    Fm = np.concatenate([np.cos(th[:, :C]), -np.sin(th[:, :C])], 0)
    G = np.concatenate([np.cos(th.T), -np.sin(th.T)], 1) / C
    G2 = np.concatenate([G[C:], G[:C]], 1)
    fill = np.full((R, 128), -np.inf, np.float32)
    for i in range(R):
        for j in range(R):
            li = 0 if (i < 8 or 16 <= i < 48) else 1
            lj = 0 if (j < 8 or 16 <= j < 48) else 1
            if li != lj:
                continue
            if i < 16 or j < 16:
                fill[i, j] = 0.0
            else:
                fill[i, j] = 0.0 if (i - 16) % 32 >= (j - 16) % 32 else -1e9
    import ml_dtypes
    return Fm.astype(np.float32).astype(ml_dtypes.bfloat16), G2.astype(np.float32).astype(ml_dtypes.bfloat16), fill


def _ln(x):
    m = jnp.mean(x, axis=-1, keepdims=True)
    xc = x - m
    v = jnp.mean(xc * xc, axis=-1, keepdims=True)
    return xc * lax.rsqrt(v + EPS)


def kernel(x_ref, mem0_ref, wqkv_hbm, wo_hbm, bk_ref, bv_ref, sh_ref, ssmk_ref, ssmd_ref,
           f_ref, g2_ref, fill_ref,
           o_ref,
           kpad_s, kv_s, u_s, kf_s, y_s, xn_s, x2_s, hn2_s, out_s, memh_s, a_s, wqkv_ref, wo_ref, sems, *, do_b=True, nsteps=NSEG + 2):
    c1 = pltpu.make_async_copy(wqkv_hbm, wqkv_ref, sems.at[0]); c1.start()
    c2 = pltpu.make_async_copy(wo_hbm, wo_ref, sems.at[1]); c2.start()
    if do_b:
        kpad_s[0:8, :] = jnp.zeros((8, D), F32)
        def cp(a, c):
            r0 = pl.multiple_of(a * C, C)
            kpad_s[pl.ds(r0 + 8, C), :] = bk_ref[pl.ds(r0, C), :].astype(F32)
            return c
        lax.fori_loop(0, NCH, cp, 0)
        sh = sh_ref[...].astype(F32)
        dd = ssmd_ref[...].astype(F32)
        fm = f_ref[...]
        for a in range(NCH):
            r0 = a * C
            ks = kpad_s[r0 + 8:r0 + 8 + C, :] * sh[0:1, :]
            for m in range(1, 4):
                ks = ks + kpad_s[r0 + 8 - m:r0 + 8 - m + C, :] * sh[m:m + 1, :]
            kv = (ks * bv_ref[r0:r0 + C, :].astype(F32)).astype(BF16)
            y_s[r0:r0 + C, :] = kv.astype(F32) * dd
            r = jnp.dot(fm, kv, preferred_element_type=F32)
            r2 = lax.dot_general(fm, ssmk_ref[:, r0:r0 + C], (((1,), (1,)), ((), ())),
                                 preferred_element_type=F32)
            for c in range(NCT):
                u_s[c, a] = r[:, c * 128:(c + 1) * 128]
                kf_s[c, a] = r2[:, c * 128:(c + 1) * 128]

        def cmac(i, carry):
            c = i // 16
            g = i % 16
            r0 = pl.multiple_of(g * 8, 8)
            r1 = pl.multiple_of(g * 8 + C, 8)
            ur = [u_s[c, a, pl.ds(r0, 8), :] for a in range(NCH)]
            ui = [u_s[c, a, pl.ds(r1, 8), :] for a in range(NCH)]
            for a in range(NCH):
                yr = None
                for j in range(a + 1):
                    kr = kf_s[c, j, pl.ds(r0, 8), :]
                    ki = kf_s[c, j, pl.ds(r1, 8), :]
                    tr = kr * ur[a - j] - ki * ui[a - j]
                    ti = kr * ui[a - j] + ki * ur[a - j]
                    if yr is None:
                        yr, yi = tr, ti
                    else:
                        yr, yi = yr + tr, yi + ti
                u_s[c, a, pl.ds(r0, 8), :] = yr
                u_s[c, a, pl.ds(r1, 8), :] = yi
            return carry
        lax.fori_loop(0, NCT * 16, cmac, 0)

        g2 = g2_ref[...]
        for c in range(NCT):
            y0 = jnp.dot(g2[:, 256:], u_s[c, 0].astype(BF16), preferred_element_type=F32)
            y_s[0:C, c * 128:(c + 1) * 128] += y0
        def inv(a, carry):
            r0 = pl.multiple_of(a * C, C)
            for c in range(NCT):
                yy = jnp.concatenate([u_s[c, a - 1], u_s[c, a]], axis=0).astype(BF16)
                y_s[pl.ds(r0, C), c * 128:(c + 1) * 128] += jnp.dot(g2, yy, preferred_element_type=F32)
            return carry
        lax.fori_loop(1, NCH, inv, 0)
    else:
        y_s[...] = jnp.zeros_like(y_s)

    def lnx(a, c):
        r0 = pl.multiple_of(a * C, C)
        xn_s[pl.ds(r0, C), :] = _ln(x_ref[pl.ds(r0, C), :].astype(F32)).astype(BF16)
        return c
    lax.fori_loop(0, NCH, lnx, 0)
    mem0f = mem0_ref[...].astype(F32)
    memh_s[...] = jnp.concatenate([mem0f, mem0f], axis=0).astype(BF16)
    out_s[...] = jnp.zeros_like(out_s)
    x2_s[0:SEG, :] = jnp.zeros((SEG, D), F32)
    hn2_s[0:SEG, :] = jnp.zeros((SEG, D), BF16)
    scale = DH ** -0.5

    c1.wait(); c2.wait()
    def seg_rows(s):
        return pl.ds(pl.multiple_of(s * SEG, SEG), SEG)

    def upd_l1(s1):
        sc = jnp.clip(s1, 0, NSEG - 1)
        x1 = x_ref[seg_rows(sc), :].astype(F32) + out_s[0:SEG, :]
        x2 = x1 + _ln(x1) * y_s[seg_rows(sc), :]
        x2_s[seg_rows(s1 + 1), :] = x2
        hn2_s[seg_rows(s1 + 1), :] = _ln(x2).astype(BF16)

    def upd_l2(s2):
        sc = jnp.clip(s2, 0, NSEG - 1)
        x3 = x2_s[seg_rows(jnp.clip(s2 + 1, 0, NSEG)), :] + out_s[SEG:2 * SEG, :]
        x4 = x3 + _ln(x3) * y_s[seg_rows(sc), :]
        o_ref[seg_rows(sc), :] = x4.astype(BF16)

    def step(t, carry):
        h = jnp.concatenate([
            memh_s[...],
            xn_s[seg_rows(jnp.minimum(t, NSEG - 1)), :],
            hn2_s[seg_rows(jnp.clip(t - 1, 0, NSEG)), :]], axis=0)
        upd_l1(t - 1)
        upd_l2(t - 3)
        fill = fill_ref[...]
        zpad = jnp.zeros((128 - R, DH), BF16)
        def proj(hd, part):
            return jnp.dot(h, wqkv_ref[hd, part], preferred_element_type=F32).astype(BF16)
        qs, ks, vs, ps, ls = {}, {}, {}, {}, {}
        def qk(i):
            s = lax.dot_general(qs.pop(i), ks.pop(i), (((1,), (1,)), ((), ())), preferred_element_type=F32)
            s = jnp.where(fill < 0, fill, s * scale)
            mx = jnp.max(s, axis=-1, keepdims=True)
            e = jnp.exp(s - mx)
            ls[i] = 1.0 / jnp.sum(e, axis=-1, keepdims=True)
            ps[i] = e.astype(BF16)
        def pv(i):
            o = jnp.dot(ps.pop(i), vs.pop(i), preferred_element_type=F32)
            a_s[:, i * DH:(i + 1) * DH] = (o * ls.pop(i)).astype(BF16)
        for hd in range(H + LAGPV):
            if hd < H:
                ks[hd] = jnp.concatenate([proj(hd, 1), zpad], axis=0)
            if 0 <= hd - 1 < H:
                qk(hd - 1)
            if hd < H:
                qs[hd] = proj(hd, 0)
                vs[hd] = jnp.concatenate([proj(hd, 2), zpad], axis=0)
            if 0 <= hd - LAGPV < H:
                pv(hd - LAGPV)
        outs = []
        for j in range(NCT):
            outs.append(jnp.dot(a_s[...], wo_ref[j], preferred_element_type=F32))
        out = jnp.concatenate(outs, axis=1)
        out_s[...] = out[16:, :]
        m2 = jnp.where(t >= 2, out[8:16, :], mem0f)
        memh_s[...] = jnp.concatenate([out[0:8, :], m2], axis=0).astype(BF16)
        return carry
    lax.fori_loop(0, nsteps, step, 0)
    upd_l2(NSEG - 1)


def make(do_b=True, nsteps=NSEG + 2):
    Fm, G2, fill = _consts()

    @jax.jit
    def run(A_x, A_mem0, A_Wq, A_Wk, A_Wv, A_Wo, B_k, B_v, B_shift_k, B_ssm_k, B_ssm_D):
        wqkv = jnp.stack([A_Wq, A_Wk, A_Wv], axis=0).transpose(2, 0, 1, 3)
        wo = A_Wo.reshape(H * DH, NCT, 128).transpose(1, 0, 2)
        out = pl.pallas_call(
            functools.partial(kernel, do_b=do_b, nsteps=nsteps),
            out_shape=jax.ShapeDtypeStruct((S, D), BF16),
            scratch_shapes=[
                pltpu.VMEM((S + 8, D), F32),
                pltpu.VMEM((S, D), BF16),
                pltpu.VMEM((NCT, NCH, 2 * C, 128), F32),
                pltpu.VMEM((NCT, NCH, 2 * C, 128), F32),
                pltpu.VMEM((S, D), F32),
                pltpu.VMEM((S, D), BF16),
                pltpu.VMEM((S + 2 * SEG, D), F32),
                pltpu.VMEM((S + 2 * SEG, D), BF16),
                pltpu.VMEM((2 * SEG, D), F32),
                pltpu.VMEM((2 * M, D), BF16),
                pltpu.VMEM((R, H * DH), BF16),
                pltpu.VMEM((H, 3, D, DH), BF16),
                pltpu.VMEM((NCT, H * DH, 128), BF16),
                pltpu.SemaphoreType.DMA((2,)),
            ],
            in_specs=[pl.BlockSpec(), pl.BlockSpec(), pl.BlockSpec(memory_space=pl.ANY), pl.BlockSpec(memory_space=pl.ANY)] + [pl.BlockSpec()] * 8,
            compiler_params=pltpu.CompilerParams(vmem_limit_bytes=120 * 1024 * 1024),
        )(A_x[0], A_mem0[0], wqkv, wo, B_k[0], B_v[0], B_shift_k.T, B_ssm_k, B_ssm_D.reshape(1, D),
          jnp.asarray(Fm), jnp.asarray(G2), jnp.asarray(fill))
        return out[None]
    return run


_RUN = make()


def pallas_interleave_layers__memory_aug_recurrent_mem_tr__ssm_conv_h3__prompt_kernel(
        A_x, A_mem0, A_Wq, A_Wk, A_Wv, A_Wo, A_seg_len, B_q, B_k, B_v, B_shift_k, B_ssm_k, B_ssm_D):
    assert int(A_seg_len) == SEG and A_x.shape == (1, S, D) and A_Wq.shape == (D, H, DH)
    del B_q
    return _RUN(A_x, A_mem0, A_Wq, A_Wk, A_Wv, A_Wo, B_k, B_v, B_shift_k, B_ssm_k, B_ssm_D)
```

```python
import functools
import numpy as np
import jax
import jax.numpy as jnp
from jax import lax
from jax.experimental import pallas as pl
from jax.experimental.pallas import tpu as pltpu

S, D, H, DH, M, SEG = 2048, 640, 32, 128, 8, 32
NSEG = S // SEG
R = 2 * (M + SEG)
C = 128
NCH = S // C
NCT = D // 128
F32, BF16, U32 = jnp.float32, jnp.bfloat16, jnp.uint32
EPS = 1e-5


def _consts():
    import ml_dtypes
    N = 2 * C
    f = np.arange(C)[:, None].astype(np.float64)
    t = np.arange(N)[None, :].astype(np.float64)
    th = np.pi * (2 * f + 1) * t / N
    Fm = np.concatenate([np.cos(th[:, :C]), -np.sin(th[:, :C])], 0)
    G = np.concatenate([np.cos(th.T), -np.sin(th.T)], 1) / C
    G2 = np.concatenate([G[C:], G[:C]], 1)
    fill = np.full((R, 128), -np.inf, np.float32)
    for i in range(R):
        for j in range(R):
            li = 0 if (i < 8 or 16 <= i < 48) else 1
            lj = 0 if (j < 8 or 16 <= j < 48) else 1
            if li != lj:
                continue
            if i < 16 or j < 16:
                fill[i, j] = 0.0
            else:
                fill[i, j] = 0.0 if (i - 16) % 32 >= (j - 16) % 32 else -1e9
    return Fm.astype(np.float32).astype(ml_dtypes.bfloat16), G2.astype(np.float32).astype(ml_dtypes.bfloat16), fill


def _ln(x):
    m = jnp.mean(x, axis=-1, keepdims=True)
    xc = x - m
    v = jnp.mean(xc * xc, axis=-1, keepdims=True)
    return xc * lax.rsqrt(v + EPS)


def _pack(x):
    return pltpu.bitcast(x.astype(BF16), U32)


def _unpack(x):
    return pltpu.bitcast(x, BF16)


def kernel(x_hbm, mem0_ref, wq_hbm, wk_hbm, wv_hbm, wo_hbm, bk_hbm, bv_hbm, sh_ref, ssmk_hbm, ssmd_ref,
           f_ref, g2_ref, fill_ref,
           o_ref,
           x_s, bk_s, bv_s, ssmk_s, raw_s, woraw_s, w32, wo32,
           kpad_s, u_s, kf_s, y_s, xn32, x2_s, hn32, out_s, memh32, a32, sems,
           *, nsteps=NSEG + 2, lagpv=2, early_dma=False):
    g1 = [pltpu.make_async_copy(bk_hbm, bk_s, sems.at[0]),
          pltpu.make_async_copy(bv_hbm, bv_s, sems.at[1]),
          pltpu.make_async_copy(ssmk_hbm, ssmk_s, sems.at[2])]
    g2 = [pltpu.make_async_copy(x_hbm, x_s, sems.at[3]),
          pltpu.make_async_copy(wq_hbm, raw_s.at[0], sems.at[4]),
          pltpu.make_async_copy(wk_hbm, raw_s.at[1], sems.at[5]),
          pltpu.make_async_copy(wv_hbm, raw_s.at[2], sems.at[6]),
          pltpu.make_async_copy(wo_hbm, woraw_s, sems.at[7])]
    for c in g1:
        c.start()
    if early_dma:
        for c in g2:
            c.start()
    kpad_s[0:8, :] = jnp.zeros((8, D), F32)
    out_s[...] = jnp.zeros_like(out_s)
    x2_s[0:SEG, :] = jnp.zeros((SEG, D), F32)
    hn32[0:SEG // 2, :] = jnp.zeros((SEG // 2, D), U32)
    g1[0].wait()

    def cp(a, c):
        r0 = pl.multiple_of(a * C, C)
        kpad_s[pl.ds(r0 + 8, C), :] = bk_s[pl.ds(r0, C), :].astype(F32)
        return c
    lax.fori_loop(0, NCH, cp, 0)
    g1[1].wait()
    g1[2].wait()
    if not early_dma:
        for c in g2:
            c.start()
    sh = sh_ref[...].astype(F32)
    dd = ssmd_ref[...].astype(F32)
    fm = f_ref[...]
    for a in range(NCH):
        r0 = a * C
        ks = kpad_s[r0 + 8:r0 + 8 + C, :] * sh[0:1, :]
        for m in range(1, 4):
            ks = ks + kpad_s[r0 + 8 - m:r0 + 8 - m + C, :] * sh[m:m + 1, :]
        kv = (ks * bv_s[r0:r0 + C, :].astype(F32)).astype(BF16)
        y_s[r0:r0 + C, :] = kv.astype(F32) * dd
        r = jnp.dot(fm, kv, preferred_element_type=F32)
        r2 = lax.dot_general(fm, ssmk_s[:, r0:r0 + C], (((1,), (1,)), ((), ())),
                             preferred_element_type=F32)
        for c in range(NCT):
            u_s[c, a] = r[:, c * 128:(c + 1) * 128]
            kf_s[c, a] = r2[:, c * 128:(c + 1) * 128]

    def cmac(i, carry):
        c = i // 16
        g = i % 16
        r0 = pl.multiple_of(g * 8, 8)
        r1 = pl.multiple_of(g * 8 + C, 8)
        ur = [u_s[c, a, pl.ds(r0, 8), :] for a in range(NCH)]
        ui = [u_s[c, a, pl.ds(r1, 8), :] for a in range(NCH)]
        for a in range(NCH):
            yr = None
            for j in range(a + 1):
                kr = kf_s[c, j, pl.ds(r0, 8), :]
                ki = kf_s[c, j, pl.ds(r1, 8), :]
                tr = kr * ur[a - j] - ki * ui[a - j]
                ti = kr * ui[a - j] + ki * ur[a - j]
                if yr is None:
                    yr, yi = tr, ti
                else:
                    yr, yi = yr + tr, yi + ti
            u_s[c, a, pl.ds(r0, 8), :] = yr
            u_s[c, a, pl.ds(r1, 8), :] = yi
        return carry
    lax.fori_loop(0, NCT * 16, cmac, 0)

    g2m = g2_ref[...]
    for c in range(NCT):
        y0 = jnp.dot(g2m[:, 256:], u_s[c, 0].astype(BF16), preferred_element_type=F32)
        y_s[0:C, c * 128:(c + 1) * 128] += y0

    def inv(a, carry):
        r0 = pl.multiple_of(a * C, C)
        for c in range(NCT):
            yy = jnp.concatenate([u_s[c, a - 1], u_s[c, a]], axis=0).astype(BF16)
            y_s[pl.ds(r0, C), c * 128:(c + 1) * 128] += jnp.dot(g2m, yy, preferred_element_type=F32)
        return carry
    lax.fori_loop(1, NCH, inv, 0)

    g2[0].wait()

    def lnx(a, c):
        r0 = pl.multiple_of(a * C, C)
        r1 = pl.multiple_of(a * (C // 2), C // 2)
        xn32[pl.ds(r1, C // 2), :] = _pack(_ln(x_s[pl.ds(r0, C), :].astype(F32)))
        return c
    lax.fori_loop(0, NCH, lnx, 0)
    mem0f = mem0_ref[...].astype(F32)
    memh32[...] = _pack(jnp.concatenate([mem0f, mem0f], axis=0))

    for part in range(3):
        g2[1 + part].wait()

        def rel(db, c, part=part):
            xw = raw_s[part, pl.ds(pl.multiple_of(db * 16, 16), 16)]
            xt = jnp.transpose(xw, (1, 0, 2))
            w32[:, part, pl.ds(pl.multiple_of(db * 8, 8), 8), :] = pltpu.bitcast(xt, U32)
            return c
        lax.fori_loop(0, D // 16, rel, 0)
    g2[4].wait()

    def relo(hd, c):
        r0 = pl.multiple_of(hd * DH, DH)
        r1 = pl.multiple_of(hd * (DH // 2), DH // 2)
        for j in range(NCT):
            wo32[j, pl.ds(r1, DH // 2), :] = pltpu.bitcast(woraw_s[pl.ds(r0, DH), j * 128:(j + 1) * 128], U32)
        return c
    lax.fori_loop(0, H, relo, 0)

    scale = DH ** -0.5

    def seg_rows(s):
        return pl.ds(pl.multiple_of(s * SEG, SEG), SEG)

    def seg_rows32(s):
        return pl.ds(pl.multiple_of(s * (SEG // 2), SEG // 2), SEG // 2)

    def upd_l1(s1):
        sc = jnp.clip(s1, 0, NSEG - 1)
        x1 = x_s[seg_rows(sc), :].astype(F32) + out_s[0:SEG, :]
        x2 = x1 + _ln(x1) * y_s[seg_rows(sc), :]
        x2_s[seg_rows(s1 + 1), :] = x2
        hn32[seg_rows32(s1 + 1), :] = _pack(_ln(x2))

    def upd_l2(s2):
        sc = jnp.clip(s2, 0, NSEG - 1)
        x3 = x2_s[seg_rows(jnp.clip(s2 + 1, 0, NSEG)), :] + out_s[SEG:2 * SEG, :]
        x4 = x3 + _ln(x3) * y_s[seg_rows(sc), :]
        o_ref[seg_rows(sc), :] = x4.astype(BF16)

    def step(t, carry):
        h = _unpack(jnp.concatenate([
            memh32[...],
            xn32[seg_rows32(jnp.minimum(t, NSEG - 1)), :],
            hn32[seg_rows32(jnp.clip(t - 1, 0, NSEG)), :]], axis=0))
        upd_l1(t - 1)
        upd_l2(t - 3)
        fill = fill_ref[...]
        zpad = jnp.zeros((128 - R, DH), F32)

        def proj(hd, part):
            return jnp.dot(h, _unpack(w32[hd, part]), preferred_element_type=F32)
        qs, ks, vs, ps, ls = {}, {}, {}, {}, {}

        def qk(i):
            s = lax.dot_general(qs.pop(i), ks.pop(i), (((1,), (1,)), ((), ())), preferred_element_type=F32)
            s = jnp.where(fill < 0, fill, s * scale)
            mx = jnp.max(s, axis=-1, keepdims=True)
            e = jnp.exp(s - mx)
            l = jnp.sum(e, axis=-1, keepdims=True)
            r = pl.reciprocal(l, approx=True)
            ls[i] = r * (2.0 - l * r)
            ps[i] = e.astype(BF16)

        def pv(i):
            o = jnp.dot(ps.pop(i), vs.pop(i), preferred_element_type=F32)
            a32[:, i * DH:(i + 1) * DH] = _pack(o * ls.pop(i))
        for hd in range(H + lagpv):
            if hd < H:
                ks[hd] = jnp.concatenate([proj(hd, 1), zpad], axis=0).astype(BF16)
            if 0 <= hd - 1 < H:
                qk(hd - 1)
            if hd < H:
                qs[hd] = proj(hd, 0).astype(BF16)
                vs[hd] = jnp.concatenate([proj(hd, 2), zpad], axis=0).astype(BF16)
            if 0 <= hd - lagpv < H:
                pv(hd - lagpv)
        outs = []
        for j in range(NCT):
            outs.append(jnp.dot(_unpack(a32[...]), _unpack(wo32[j]), preferred_element_type=F32))
        out = jnp.concatenate(outs, axis=1)
        out_s[...] = out[16:, :]
        m2 = jnp.where(t >= 2, out[8:16, :], mem0f)
        memh32[...] = _pack(jnp.concatenate([out[0:8, :], m2], axis=0))
        return carry
    lax.fori_loop(0, nsteps, step, 0)
    upd_l2(NSEG - 1)


def make(**kw):
    Fm, G2, fill = _consts()

    @jax.jit
    def run(A_x, A_mem0, A_Wq, A_Wk, A_Wv, A_Wo, B_k, B_v, B_shift_k, B_ssm_k, B_ssm_D):
        hbm = pl.BlockSpec(memory_space=pltpu.HBM)
        vm = pl.BlockSpec()
        out = pl.pallas_call(
            functools.partial(kernel, **kw),
            out_shape=jax.ShapeDtypeStruct((S, D), BF16),
            in_specs=[hbm, vm, hbm, hbm, hbm, hbm, hbm, hbm, vm, hbm, vm, vm, vm, vm],
            scratch_shapes=[
                pltpu.VMEM((S, D), BF16),
                pltpu.VMEM((S, D), BF16),
                pltpu.VMEM((S, D), BF16),
                pltpu.VMEM((D, S), BF16),
                pltpu.VMEM((3, D, H, DH), BF16),
                pltpu.VMEM((H * DH, D), BF16),
                pltpu.VMEM((H, 3, D // 2, DH), U32),
                pltpu.VMEM((NCT, H * DH // 2, 128), U32),
                pltpu.VMEM((S + 8, D), F32),
                pltpu.VMEM((NCT, NCH, 2 * C, 128), F32),
                pltpu.VMEM((NCT, NCH, 2 * C, 128), F32),
                pltpu.VMEM((S, D), F32),
                pltpu.VMEM((S // 2, D), U32),
                pltpu.VMEM((S + 2 * SEG, D), F32),
                pltpu.VMEM((S // 2 + SEG, D), U32),
                pltpu.VMEM((2 * SEG, D), F32),
                pltpu.VMEM((M, D), U32),
                pltpu.VMEM((R // 2, H * DH), U32),
                pltpu.SemaphoreType.DMA((8,)),
            ],
            compiler_params=pltpu.CompilerParams(vmem_limit_bytes=120 * 1024 * 1024),
        )(A_x.reshape(S, D), A_mem0.reshape(M, D), A_Wq, A_Wk, A_Wv, A_Wo.reshape(H * DH, D),
          B_k.reshape(S, D), B_v.reshape(S, D), B_shift_k.T, B_ssm_k, B_ssm_D.reshape(1, D),
          jnp.asarray(Fm), jnp.asarray(G2), jnp.asarray(fill))
        return out.reshape(1, S, D)
    return run


_RUN = make()


def pallas_interleave_layers__memory_aug_recurrent_mem_tr__ssm_conv_h3__prompt_kernel(
        A_x, A_mem0, A_Wq, A_Wk, A_Wv, A_Wo, A_seg_len, B_q, B_k, B_v, B_shift_k, B_ssm_k, B_ssm_D):
    assert int(A_seg_len) == SEG and A_x.shape == (1, S, D) and A_Wq.shape == (D, H, DH)
    del B_q
    return _RUN(A_x, A_mem0, A_Wq, A_Wk, A_Wv, A_Wo, B_k, B_v, B_shift_k, B_ssm_k, B_ssm_D)
```

```python
import functools
import numpy as np
import jax
import jax.numpy as jnp
from jax import lax
from jax.experimental import pallas as pl
from jax.experimental.pallas import tpu as pltpu

S, D, H, DH, M, SEG = 2048, 640, 32, 128, 8, 32
NSEG = S // SEG
R = 2 * (M + SEG)
C = 128
NCH = S // C
NCT = D // 128
F32, BF16, U32 = jnp.float32, jnp.bfloat16, jnp.uint32
EPS = 1e-5


def _consts():
    import ml_dtypes
    N = 2 * C
    f = np.arange(C)[:, None].astype(np.float64)
    t = np.arange(N)[None, :].astype(np.float64)
    th = np.pi * (2 * f + 1) * t / N
    Fm = np.concatenate([np.cos(th[:, :C]), -np.sin(th[:, :C])], 0)
    G = np.concatenate([np.cos(th.T), -np.sin(th.T)], 1) / C
    G2 = np.concatenate([G[C:], G[:C]], 1)
    fill = np.full((R, 128), -np.inf, np.float32)
    for i in range(R):
        for j in range(R):
            li = 0 if (i < 8 or 16 <= i < 48) else 1
            lj = 0 if (j < 8 or 16 <= j < 48) else 1
            if li != lj:
                continue
            if i < 16 or j < 16:
                fill[i, j] = 0.0
            else:
                fill[i, j] = 0.0 if (i - 16) % 32 >= (j - 16) % 32 else -1e9
    RL = 2 * M + SEG
    fill2 = np.full((2, RL, 128), -np.inf, np.float32)
    for l in range(2):
        for i in range(RL):
            for j in range(RL):
                if j < 16:
                    if j // 8 == l:
                        fill2[l, i, j] = 0.0
                elif i < 16:
                    fill2[l, i, j] = 0.0
                else:
                    fill2[l, i, j] = 0.0 if i >= j else -1e9
    return (Fm.astype(np.float32).astype(ml_dtypes.bfloat16), G2.astype(np.float32).astype(ml_dtypes.bfloat16),
            fill, fill2)


def _ln(x):
    m = jnp.mean(x, axis=-1, keepdims=True)
    xc = x - m
    v = jnp.mean(xc * xc, axis=-1, keepdims=True)
    return xc * lax.rsqrt(v + EPS)


def _pack(x):
    return pltpu.bitcast(x.astype(BF16), U32)


def _unpack(x):
    return pltpu.bitcast(x, BF16)


def kernel(x_hbm, mem0_ref, wq_hbm, wk_hbm, wv_hbm, wo_hbm, bk_hbm, bv_hbm, sh_ref, ssmk_hbm, ssmd_ref,
           f_ref, g2_ref, fill_ref, fill2_ref,
           o_ref,
           x_s, bk_s, bv_s, ssmk_s, raw_s, woraw_s, w32, wo32,
           u_s, kf_s, y_s, xn32, x2_s, hn32, out_s, memh32, a32, sems,
           *, nsteps=NSEG + 2, lagpv=2, tailfill=True, light=True, lagqk_l=2, lagpv_l=4, unroll=2, nfill=28, split=True, ndma_early=8, cmac_unroll=1, kfwd_mode=0, LNB=256):
    srcs = [(bk_hbm, bk_s), (bv_hbm, bv_s), (ssmk_hbm, ssmk_s), (x_hbm, x_s),
            (wq_hbm, raw_s.at[0]), (wk_hbm, raw_s.at[1]), (wv_hbm, raw_s.at[2]), (wo_hbm, woraw_s)]
    cps = [pltpu.make_async_copy(a_, b_, sems.at[i]) for i, (a_, b_) in enumerate(srcs)]
    for c in cps[:ndma_early]:
        c.start()
    out_s[...] = jnp.zeros_like(out_s)
    x2_s[0:SEG, :] = jnp.zeros((SEG, D), F32)
    hn32[0:SEG // 2, :] = jnp.zeros((SEG // 2, D), U32)
    mem0f = mem0_ref[...].astype(F32)
    memh32[...] = _pack(jnp.concatenate([mem0f, mem0f], axis=0))
    sh = sh_ref[...].astype(F32)
    dd = ssmd_ref[...].astype(F32)
    fm = f_ref[...]
    cps[0].wait()
    cps[1].wait()
    for c in cps[ndma_early:]:
        c.start()

    prev = [jnp.zeros((8, 128), F32)] * NCT
    for a in range(NCH):
        r0 = a * C
        for c in range(NCT):
            cs = slice(c * 128, (c + 1) * 128)
            cur = bk_s[r0:r0 + C, cs].astype(F32)
            ext = jnp.concatenate([prev[c], cur], axis=0)
            ks = cur * sh[0:1, cs]
            for m in range(1, 4):
                ks = ks + ext[8 - m:8 - m + C, :] * sh[m:m + 1, cs]
            prev[c] = cur[C - 8:, :]
            kv = (ks * bv_s[r0:r0 + C, cs].astype(F32)).astype(BF16)
            y_s[r0:r0 + C, cs] = kv.astype(F32) * dd[:, cs]
            u_s[c, a] = jnp.dot(fm, kv, preferred_element_type=F32)
        if kfwd_mode == 1:
            if a == 0:
                cps[2].wait()
            for c in range(NCT):
                kf_s[c, a] = lax.dot_general(fm, ssmk_s[c * 128:(c + 1) * 128, r0:r0 + C], (((1,), (1,)), ((), ())),
                                             preferred_element_type=F32)
    if kfwd_mode == 0:
        cps[2].wait()
        for a in range(NCH):
            r0 = a * C
            for c in range(NCT):
                kf_s[c, a] = lax.dot_general(fm, ssmk_s[c * 128:(c + 1) * 128, r0:r0 + C], (((1,), (1,)), ((), ())),
                                             preferred_element_type=F32)

    cps[3].wait()

    def lnx(a, c):
        r0 = pl.multiple_of(a * LNB, LNB)
        r1 = pl.multiple_of(a * (LNB // 2), LNB // 2)
        xn32[pl.ds(r1, LNB // 2), :] = _pack(_ln(x_s[pl.ds(r0, LNB), :].astype(F32)))
        return c
    lax.fori_loop(0, S // LNB, lnx, 0)

    def cmac(i, carry):
        c = i // 16
        g = i % 16
        r0 = pl.multiple_of(g * 8, 8)
        r1 = pl.multiple_of(g * 8 + C, 8)
        ur = [u_s[c, a, pl.ds(r0, 8), :] for a in range(NCH)]
        ui = [u_s[c, a, pl.ds(r1, 8), :] for a in range(NCH)]
        for a in range(NCH):
            yr = None
            for j in range(a + 1):
                kr = kf_s[c, j, pl.ds(r0, 8), :]
                ki = kf_s[c, j, pl.ds(r1, 8), :]
                tr = kr * ur[a - j] - ki * ui[a - j]
                ti = kr * ui[a - j] + ki * ur[a - j]
                if yr is None:
                    yr, yi = tr, ti
                else:
                    yr, yi = yr + tr, yi + ti
            u_s[c, a, pl.ds(r0, 8), :] = yr
            u_s[c, a, pl.ds(r1, 8), :] = yi
        return carry
    lax.fori_loop(0, NCT * 16, cmac, 0, unroll=cmac_unroll)

    def rel_block(part, db):
        r0 = pl.multiple_of(db * 8, 8)
        e = pltpu.bitcast(raw_s[part, db, :, 0], U32)
        o = pltpu.bitcast(raw_s[part, db, :, 1], U32)
        lo = jnp.transpose((e & 0xFFFF) | (o << 16), (1, 0, 2))
        hi = jnp.transpose((e >> 16) | (o & np.uint32(0xFFFF0000)), (1, 0, 2))
        for hp in range(H // 2):
            w32[2 * hp, part, pl.ds(r0, 8), :] = lo[hp]
            w32[2 * hp + 1, part, pl.ds(r0, 8), :] = hi[hp]

    g2m = g2_ref[...]
    NDB = D // 16
    cps[4].wait()
    for c in range(NCT):
        y0 = jnp.dot(g2m[:, 256:], u_s[c, 0].astype(BF16), preferred_element_type=F32)
        y_s[0:C, c * 128:(c + 1) * 128] += y0
        rel_block(0, c)

    def inv(a, carry):
        r0 = pl.multiple_of(a * C, C)
        part = a >> 3
        db0 = (a & 7) * 5
        for c in range(NCT):
            yy = jnp.concatenate([u_s[c, a - 1], u_s[c, a]], axis=0).astype(BF16)
            y_s[pl.ds(r0, C), c * 128:(c + 1) * 128] += jnp.dot(g2m, yy, preferred_element_type=F32)
            rel_block(part, db0 + c)
        return carry
    lax.fori_loop(1, 8, inv, 0)
    cps[5].wait()
    lax.fori_loop(8, NCH, inv, 0)

    def rel_range(part, lo_, hi_):
        def body(db, c):
            rel_block(part, db)
            return c
        lax.fori_loop(lo_, hi_, body, 0, unroll=2)
    cps[6].wait()
    rel_range(2, 0, NDB)
    cps[7].wait()

    def relo(hd, c):
        r0 = pl.multiple_of(hd * DH, DH)
        r1 = pl.multiple_of(hd * (DH // 2), DH // 2)
        for j in range(NCT):
            wo32[j, pl.ds(r1, DH // 2), :] = pltpu.bitcast(woraw_s[pl.ds(r0, DH), j * 128:(j + 1) * 128], U32)
        return c
    lax.fori_loop(0, H, relo, 0)

    scale = DH ** -0.5

    def seg_rows(s):
        return pl.ds(pl.multiple_of(s * SEG, SEG), SEG)

    def seg_rows32(s):
        return pl.ds(pl.multiple_of(s * (SEG // 2), SEG // 2), SEG // 2)

    def upd_l1(s1):
        sc = jnp.clip(s1, 0, NSEG - 1)
        x1 = x_s[seg_rows(sc), :].astype(F32) + out_s[0:SEG, :]
        x2 = x1 + _ln(x1) * y_s[seg_rows(sc), :]
        x2_s[seg_rows(s1 + 1), :] = x2
        hn32[seg_rows32(s1 + 1), :] = _pack(_ln(x2))

    def upd_l2(s2):
        sc = jnp.clip(s2, 0, NSEG - 1)
        x3 = x2_s[seg_rows(jnp.clip(s2 + 1, 0, NSEG)), :] + out_s[SEG:2 * SEG, :]
        x4 = x3 + _ln(x3) * y_s[seg_rows(sc), :]
        o_ref[seg_rows(sc), :] = x4.astype(BF16)

    def attn_block(h, fill, nrow, lagqk, lagpv_):
        zpad = jnp.zeros((128 - nrow, DH), F32)
        nr2 = nrow // 2

        def proj(hd, part):
            return jnp.dot(h, _unpack(w32[hd, part]), preferred_element_type=F32)
        qs, ks, vs, ps, ls = {}, {}, {}, {}, {}

        def qk(i):
            s_ = lax.dot_general(qs.pop(i), ks.pop(i), (((1,), (1,)), ((), ())), preferred_element_type=F32)
            s_ = jnp.where(fill < 0, fill, s_ * scale)
            mx = jnp.max(s_, axis=-1, keepdims=True)
            e = jnp.exp(s_ - mx)
            l = jnp.sum(e, axis=-1, keepdims=True)
            r = pl.reciprocal(l, approx=True)
            ls[i] = r * (2.0 - l * r)
            ps[i] = e.astype(BF16)

        def pv(i):
            o = jnp.dot(ps.pop(i), vs.pop(i), preferred_element_type=F32)
            a32[0:nr2, i * DH:(i + 1) * DH] = _pack(o * ls.pop(i))
        acc = {}

        def p2(j, h0, h1):
            r = jnp.dot(_unpack(a32[0:nr2, h0 * DH:h1 * DH]), _unpack(wo32[j, h0 * (DH // 2):h1 * (DH // 2), :]),
                        preferred_element_type=F32)
            acc[j] = r if j not in acc else acc[j] + r
        done = [0] * NCT

        def fill_p2(n, ready):
            for j in range(NCT):
                if n <= 0:
                    break
                k_ = min(n, ready - done[j])
                if k_ > 0:
                    p2(j, done[j], done[j] + k_)
                    done[j] += k_
                    n -= k_
                    if done[j] < ready and n <= 0:
                        break
        for hd in range(H + lagpv_):
            tail = tailfill and hd >= H
            rdy = max(hd - lagpv_ - 1, 0)
            if hd < H:
                ks[hd] = jnp.concatenate([proj(hd, 1), zpad], axis=0).astype(BF16)
            elif tail:
                fill_p2(5, rdy)
            if 0 <= hd - lagqk < H:
                qk(hd - lagqk)
            if hd < H:
                qs[hd] = proj(hd, 0).astype(BF16)
                vs[hd] = jnp.concatenate([proj(hd, 2), zpad], axis=0).astype(BF16)
            elif tail:
                fill_p2(10, rdy)
            if 0 <= hd - lagpv_ < H:
                pv(hd - lagpv_)
        if tailfill:
            fill_p2(nfill, H - 1)
        for j in range(NCT):
            if done[j] < H:
                p2(j, done[j], H)
        return [acc[j] for j in range(NCT)]

    def step_full(t):
        h = _unpack(jnp.concatenate([
            memh32[...],
            xn32[seg_rows32(jnp.minimum(t, NSEG - 1)), :],
            hn32[seg_rows32(jnp.clip(t - 1, 0, NSEG)), :]], axis=0))
        upd_l1(t - 1)
        upd_l2(t - 3)
        outs = attn_block(h, fill_ref[...], R, 1, lagpv)
        out = jnp.concatenate(outs, axis=1)
        out_s[...] = out[16:, :]
        if light:
            memh32[...] = _pack(out[0:16, :])
        else:
            m2 = jnp.where(t >= 2, out[8:16, :], mem0f)
            memh32[...] = _pack(jnp.concatenate([out[0:8, :], m2], axis=0))

    def step_light(t):
        lay = (t >= 2).astype(jnp.int32)
        mold = memh32[...]
        tok = jnp.where(lay == 1, hn32[seg_rows32(jnp.clip(t - 1, 0, NSEG)), :],
                        xn32[seg_rows32(jnp.minimum(t, NSEG - 1)), :])
        h = _unpack(jnp.concatenate([mold, tok], axis=0))
        upd_l1(t - 1)
        upd_l2(t - 3)
        outs = attn_block(h, fill2_ref[lay], 2 * M + SEG, lagqk_l, lagpv_l)
        out = jnp.concatenate(outs, axis=1)
        out_s[seg_rows(lay), :] = out[16:, :]
        rowl = lax.broadcasted_iota(jnp.int32, (M, D), 0) >> 2
        memh32[...] = jnp.where(rowl == lay, _pack(out[0:16, :]), mold)

    if light and split:
        def stepl(t, carry):
            step_light(t)
            return carry

        def stepf(t, carry):
            step_full(t)
            return carry
        lax.fori_loop(0, 2, stepl, 0)
        lax.fori_loop(2, NSEG, stepf, 0, unroll=unroll)
        lax.fori_loop(NSEG, NSEG + 2, stepl, 0)
    elif light:
        def step(t, carry):
            is_light = jnp.logical_or(t < 2, t >= NSEG)

            @pl.when(is_light)
            def _():
                step_light(t)

            @pl.when(jnp.logical_not(is_light))
            def _():
                step_full(t)
            return carry
        lax.fori_loop(0, nsteps, step, 0)
    else:
        def step(t, carry):
            step_full(t)
            return carry
        lax.fori_loop(0, nsteps, step, 0, unroll=unroll)
    upd_l2(NSEG - 1)


def make(**kw):
    Fm, G2, fill, fill2 = _consts()

    @jax.jit
    def run(A_x, A_mem0, A_Wq, A_Wk, A_Wv, A_Wo, B_k, B_v, B_shift_k, B_ssm_k, B_ssm_D):
        hbm = pl.BlockSpec(memory_space=pltpu.HBM)
        vm = pl.BlockSpec()
        wr = lambda w: w.reshape(D // 16, 8, 2, H, DH)
        out = pl.pallas_call(
            functools.partial(kernel, **kw),
            out_shape=jax.ShapeDtypeStruct((S, D), BF16),
            in_specs=[hbm, vm, hbm, hbm, hbm, hbm, hbm, hbm, vm, hbm, vm, vm, vm, vm, vm],
            scratch_shapes=[
                pltpu.VMEM((S, D), BF16),
                pltpu.VMEM((S, D), BF16),
                pltpu.VMEM((S, D), BF16),
                pltpu.VMEM((D, S), BF16),
                pltpu.VMEM((3, D // 16, 8, 2, H, DH), BF16),
                pltpu.VMEM((H * DH, D), BF16),
                pltpu.VMEM((H, 3, D // 2, DH), U32),
                pltpu.VMEM((NCT, H * DH // 2, 128), U32),
                pltpu.VMEM((NCT, NCH, 2 * C, 128), F32),
                pltpu.VMEM((NCT, NCH, 2 * C, 128), F32),
                pltpu.VMEM((S, D), F32),
                pltpu.VMEM((S // 2, D), U32),
                pltpu.VMEM((S + 2 * SEG, D), F32),
                pltpu.VMEM((S // 2 + SEG, D), U32),
                pltpu.VMEM((2 * SEG, D), F32),
                pltpu.VMEM((M, D), U32),
                pltpu.VMEM((R // 2, H * DH), U32),
                pltpu.SemaphoreType.DMA((8,)),
            ],
            compiler_params=pltpu.CompilerParams(vmem_limit_bytes=120 * 1024 * 1024),
        )(A_x.reshape(S, D), A_mem0.reshape(M, D), wr(A_Wq), wr(A_Wk), wr(A_Wv), A_Wo.reshape(H * DH, D),
          B_k.reshape(S, D), B_v.reshape(S, D), B_shift_k.T, B_ssm_k, B_ssm_D.reshape(1, D),
          jnp.asarray(Fm), jnp.asarray(G2), jnp.asarray(fill), jnp.asarray(fill2))
        return out.reshape(1, S, D)
    return run


_RUN = make()


def pallas_interleave_layers__memory_aug_recurrent_mem_tr__ssm_conv_h3__prompt_kernel(
        A_x, A_mem0, A_Wq, A_Wk, A_Wv, A_Wo, A_seg_len, B_q, B_k, B_v, B_shift_k, B_ssm_k, B_ssm_D):
    assert int(A_seg_len) == SEG and A_x.shape == (1, S, D) and A_Wq.shape == (D, H, DH)
    del B_q
    return _RUN(A_x, A_mem0, A_Wq, A_Wk, A_Wv, A_Wo, B_k, B_v, B_shift_k, B_ssm_k, B_ssm_D)
```

```python
import functools
import numpy as np
import jax
import jax.numpy as jnp
from jax import lax
from jax.experimental import pallas as pl
from jax.experimental.pallas import tpu as pltpu

S, D, H, DH, M, SEG = 2048, 640, 32, 128, 8, 32
NSEG = S // SEG
R = 2 * (M + SEG)
C = 128
NCH = S // C
NCT = D // 128
F32, BF16, U32 = jnp.float32, jnp.bfloat16, jnp.uint32
EPS = 1e-5


def _consts():
    import ml_dtypes
    N = 2 * C
    f = np.arange(C)[:, None].astype(np.float64)
    t = np.arange(N)[None, :].astype(np.float64)
    th = np.pi * (2 * f + 1) * t / N
    Fm = np.concatenate([np.cos(th[:, :C]), -np.sin(th[:, :C])], 0)
    G = np.concatenate([np.cos(th.T), -np.sin(th.T)], 1) / C
    G2 = np.concatenate([G[C:], G[:C]], 1)
    fill = np.full((R, 128), -np.inf, np.float32)
    for i in range(R):
        for j in range(R):
            li = 0 if (i < 8 or 16 <= i < 48) else 1
            lj = 0 if (j < 8 or 16 <= j < 48) else 1
            if li != lj:
                continue
            if i < 16 or j < 16:
                fill[i, j] = 0.0
            else:
                fill[i, j] = 0.0 if (i - 16) % 32 >= (j - 16) % 32 else -1e9
    RL = 2 * M + SEG
    fill2 = np.full((2, RL, 128), -np.inf, np.float32)
    for l in range(2):
        for i in range(RL):
            for j in range(RL):
                if j < 16:
                    if j // 8 == l:
                        fill2[l, i, j] = 0.0
                elif i < 16:
                    fill2[l, i, j] = 0.0
                else:
                    fill2[l, i, j] = 0.0 if i >= j else -1e9
    return (Fm.astype(np.float32).astype(ml_dtypes.bfloat16), G2.astype(np.float32).astype(ml_dtypes.bfloat16),
            fill, fill2)


def _ln(x):
    m = jnp.mean(x, axis=-1, keepdims=True)
    xc = x - m
    v = jnp.mean(xc * xc, axis=-1, keepdims=True)
    return xc * lax.rsqrt(v + EPS)


def _pack(x):
    return pltpu.bitcast(x.astype(BF16), U32)


def _unpack(x):
    return pltpu.bitcast(x, BF16)


def kernel(x_hbm, mem0_ref, wq_hbm, wk_hbm, wv_hbm, wo_hbm, bk_hbm, bv_hbm, sh_ref, ssmk_hbm, ssmd_ref,
           f_ref, g2_ref, fill_ref, fill2_ref,
           o_ref,
           o_s_b, x_s, bk_s, bv_s, ssmk_s, raw_s, woraw_s, w32, wo32,
           u_s, kf_s, y_s, xn32, x2_s, hn32, out_s, memh32, a32, o_s_a, sems,
           *, nfull=NSEG - 2, ospos=0, lagpv=2, tailfill=True, lagqk_l=2, lagpv_l=4, unroll=2, nfill=28, rmargin=2, nspl=2, ln_inloop=True, ostream=True, cmac_unroll=2, kfwd_mode=0, LNB=256):
    o_s = o_s_a if ospos == 0 else o_s_b
    PR = S // nspl
    kvc = []
    for i in range(nspl):
        rs = pl.ds(i * PR, PR)
        kvc.append((pltpu.make_async_copy(bk_hbm.at[rs], bk_s.at[rs], sems.at[8 + 2 * i]),
                    pltpu.make_async_copy(bv_hbm.at[rs], bv_s.at[rs], sems.at[8 + 2 * i + 1])))
    srcs = [None, None, (ssmk_hbm, ssmk_s), (x_hbm, x_s),
            (wq_hbm, raw_s.at[0]), (wk_hbm, raw_s.at[1]), (wv_hbm, raw_s.at[2]), (wo_hbm, woraw_s)]
    cps = [None, None] + [pltpu.make_async_copy(a_, b_, sems.at[i + 2]) for i, (a_, b_) in enumerate(srcs[2:])]
    for c0, c1 in kvc:
        c0.start()
        c1.start()
    for c in cps[2:]:
        c.start()
    out_s[...] = jnp.zeros_like(out_s)
    x2_s[0:SEG, :] = jnp.zeros((SEG, D), F32)
    hn32[0:SEG // 2, :] = jnp.zeros((SEG // 2, D), U32)
    mem0f = mem0_ref[...].astype(F32)
    memh32[...] = _pack(jnp.concatenate([mem0f, mem0f], axis=0))
    sh = sh_ref[...].astype(F32)
    dd = ssmd_ref[...].astype(F32)
    fm = f_ref[...]

    prev = [jnp.zeros((8, 128), F32)] * NCT
    for a in range(NCH):
        r0 = a * C
        if r0 % PR == 0:
            kvc[r0 // PR][0].wait()
            kvc[r0 // PR][1].wait()
        for c in range(NCT):
            cs = slice(c * 128, (c + 1) * 128)
            cur = bk_s[r0:r0 + C, cs].astype(F32)
            ext = jnp.concatenate([prev[c], cur], axis=0)
            ks = cur * sh[0:1, cs]
            for m in range(1, 4):
                ks = ks + ext[8 - m:8 - m + C, :] * sh[m:m + 1, cs]
            prev[c] = cur[C - 8:, :]
            kv = (ks * bv_s[r0:r0 + C, cs].astype(F32)).astype(BF16)
            y_s[r0:r0 + C, cs] = kv.astype(F32) * dd[:, cs]
            u_s[c, a] = jnp.dot(fm, kv, preferred_element_type=F32)
        if kfwd_mode == 1:
            if a == 0:
                cps[2].wait()
            for c in range(NCT):
                kf_s[c, a] = lax.dot_general(fm, ssmk_s[c * 128:(c + 1) * 128, r0:r0 + C], (((1,), (1,)), ((), ())),
                                             preferred_element_type=F32)
    if kfwd_mode == 0:
        cps[2].wait()
        for a in range(NCH):
            r0 = a * C
            for c in range(NCT):
                kf_s[c, a] = lax.dot_general(fm, ssmk_s[c * 128:(c + 1) * 128, r0:r0 + C], (((1,), (1,)), ((), ())),
                                             preferred_element_type=F32)

    cps[3].wait()

    if ln_inloop:
        xn32[0:SEG // 2, :] = _pack(_ln(x_s[0:SEG, :].astype(F32)))
    else:
        def lnx(a, c):
            r0 = pl.multiple_of(a * LNB, LNB)
            r1 = pl.multiple_of(a * (LNB // 2), LNB // 2)
            xn32[pl.ds(r1, LNB // 2), :] = _pack(_ln(x_s[pl.ds(r0, LNB), :].astype(F32)))
            return c
        lax.fori_loop(0, S // LNB, lnx, 0)

    def cmac(i, carry):
        c = i // 16
        g = i % 16
        r0 = pl.multiple_of(g * 8, 8)
        r1 = pl.multiple_of(g * 8 + C, 8)
        ur = [u_s[c, a, pl.ds(r0, 8), :] for a in range(NCH)]
        ui = [u_s[c, a, pl.ds(r1, 8), :] for a in range(NCH)]
        for a in range(NCH):
            yr = None
            for j in range(a + 1):
                kr = kf_s[c, j, pl.ds(r0, 8), :]
                ki = kf_s[c, j, pl.ds(r1, 8), :]
                tr = kr * ur[a - j] - ki * ui[a - j]
                ti = kr * ui[a - j] + ki * ur[a - j]
                if yr is None:
                    yr, yi = tr, ti
                else:
                    yr, yi = yr + tr, yi + ti
            u_s[c, a, pl.ds(r0, 8), :] = yr
            u_s[c, a, pl.ds(r1, 8), :] = yi
        return carry
    lax.fori_loop(0, NCT * 16, cmac, 0, unroll=cmac_unroll)

    def rel_block(part, db):
        r0 = pl.multiple_of(db * 8, 8)
        e = pltpu.bitcast(raw_s[part, db, :, 0], U32)
        o = pltpu.bitcast(raw_s[part, db, :, 1], U32)
        lo = jnp.transpose((e & 0xFFFF) | (o << 16), (1, 0, 2))
        hi = jnp.transpose((e >> 16) | (o & np.uint32(0xFFFF0000)), (1, 0, 2))
        for hp in range(H // 2):
            w32[2 * hp, part, pl.ds(r0, 8), :] = lo[hp]
            w32[2 * hp + 1, part, pl.ds(r0, 8), :] = hi[hp]

    g2m = g2_ref[...]
    NDB = D // 16
    cps[4].wait()
    for c in range(NCT):
        y0 = jnp.dot(g2m[:, 256:], u_s[c, 0].astype(BF16), preferred_element_type=F32)
        y_s[0:C, c * 128:(c + 1) * 128] += y0
        rel_block(0, c)

    def inv(a, carry):
        r0 = pl.multiple_of(a * C, C)
        part = a >> 3
        db0 = (a & 7) * 5
        for c in range(NCT):
            yy = jnp.concatenate([u_s[c, a - 1], u_s[c, a]], axis=0).astype(BF16)
            y_s[pl.ds(r0, C), c * 128:(c + 1) * 128] += jnp.dot(g2m, yy, preferred_element_type=F32)
            rel_block(part, db0 + c)
        return carry
    lax.fori_loop(1, 8, inv, 0)
    cps[5].wait()
    lax.fori_loop(8, NCH, inv, 0)

    def rel_range(part, lo_, hi_):
        def body(db, c):
            rel_block(part, db)
            return c
        lax.fori_loop(lo_, hi_, body, 0, unroll=2)
    cps[6].wait()
    rel_range(2, 0, NDB)
    cps[7].wait()

    def relo(hd, c):
        r0 = pl.multiple_of(hd * DH, DH)
        r1 = pl.multiple_of(hd * (DH // 2), DH // 2)
        for j in range(NCT):
            wo32[j, pl.ds(r1, DH // 2), :] = pltpu.bitcast(woraw_s[pl.ds(r0, DH), j * 128:(j + 1) * 128], U32)
        return c
    lax.fori_loop(0, H, relo, 0)

    scale = DH ** -0.5

    def seg_rows(s):
        return pl.ds(pl.multiple_of(s * SEG, SEG), SEG)

    def seg_rows32(s):
        return pl.ds(pl.multiple_of(s * (SEG // 2), SEG // 2), SEG // 2)

    def upd_l1(s1):
        sc = jnp.clip(s1, 0, NSEG - 1)
        x1 = x_s[seg_rows(sc), :].astype(F32) + out_s[0:SEG, :]
        x2 = x1 + _ln(x1) * y_s[seg_rows(sc), :]
        x2_s[seg_rows(s1 + 1), :] = x2
        hn32[seg_rows32(s1 + 1), :] = _pack(_ln(x2))

    def ln_next(t):
        if ln_inloop:
            xn32[seg_rows32(jnp.minimum(t + 1, NSEG)), :] = _pack(
                _ln(x_s[seg_rows(jnp.minimum(t + 1, NSEG - 1)), :].astype(F32)))

    def ocopy(u):
        return pltpu.make_async_copy(o_s.at[seg_rows(u)], o_ref.at[seg_rows(u)], sems.at[0])

    def upd_l2(s2):
        sc = jnp.clip(s2, 0, NSEG - 1)
        x3 = x2_s[seg_rows(jnp.clip(s2 + 1, 0, NSEG)), :] + out_s[SEG:2 * SEG, :]
        x4 = x3 + _ln(x3) * y_s[seg_rows(sc), :]
        (o_s if ostream else o_ref)[seg_rows(sc), :] = x4.astype(BF16)

    def attn_block(h, fill, nrow, lagqk, lagpv_):
        zpad = jnp.zeros((128 - nrow, DH), F32)
        nr2 = nrow // 2

        def proj(hd, part):
            return jnp.dot(h, _unpack(w32[hd, part]), preferred_element_type=F32)
        qs, ks, vs, ps, ls = {}, {}, {}, {}, {}

        def qk(i):
            s_ = lax.dot_general(qs.pop(i), ks.pop(i), (((1,), (1,)), ((), ())), preferred_element_type=F32)
            s_ = jnp.where(fill < 0, fill, s_ * scale)
            mx = jnp.max(s_, axis=-1, keepdims=True)
            e = jnp.exp(s_ - mx)
            l = jnp.sum(e, axis=-1, keepdims=True)
            r = pl.reciprocal(l, approx=True)
            ls[i] = r * (2.0 - l * r)
            ps[i] = e.astype(BF16)

        def pv(i):
            o = jnp.dot(ps.pop(i), vs.pop(i), preferred_element_type=F32)
            a32[0:nr2, i * DH:(i + 1) * DH] = _pack(o * ls.pop(i))
        acc = {}

        def p2(j, h0, h1):
            r = jnp.dot(_unpack(a32[0:nr2, h0 * DH:h1 * DH]), _unpack(wo32[j, h0 * (DH // 2):h1 * (DH // 2), :]),
                        preferred_element_type=F32)
            acc[j] = r if j not in acc else acc[j] + r
        done = [0] * NCT

        def fill_p2(n, ready):
            for j in range(NCT):
                if n <= 0:
                    break
                k_ = min(n, ready - done[j])
                if k_ > 0:
                    p2(j, done[j], done[j] + k_)
                    done[j] += k_
                    n -= k_
                    if done[j] < ready and n <= 0:
                        break
        for hd in range(H + lagpv_):
            tail = tailfill and hd >= H
            rdy = max(hd - lagpv_ - rmargin, 0)
            if hd < H:
                ks[hd] = jnp.concatenate([proj(hd, 1), zpad], axis=0).astype(BF16)
            elif tail:
                fill_p2(5, rdy)
            if 0 <= hd - lagqk < H:
                qk(hd - lagqk)
            if hd < H:
                qs[hd] = proj(hd, 0).astype(BF16)
                vs[hd] = jnp.concatenate([proj(hd, 2), zpad], axis=0).astype(BF16)
            elif tail:
                fill_p2(10, rdy)
            if 0 <= hd - lagpv_ < H:
                pv(hd - lagpv_)
        if tailfill:
            fill_p2(nfill, H - rmargin)
        for j in range(NCT):
            if done[j] < H:
                p2(j, done[j], H)
        return [acc[j] for j in range(NCT)]

    def step_full(t):
        if ostream:
            @pl.when(t >= 4)
            def _():
                ocopy(t - 4).start()
        h = _unpack(jnp.concatenate([
            memh32[...],
            xn32[seg_rows32(jnp.minimum(t, NSEG - 1)), :],
            hn32[seg_rows32(jnp.clip(t - 1, 0, NSEG)), :]], axis=0))
        upd_l1(t - 1)
        upd_l2(t - 3)
        ln_next(t)
        outs = attn_block(h, fill_ref[...], R, 1, lagpv)
        out = jnp.concatenate(outs, axis=1)
        out_s[...] = out[16:, :]
        memh32[...] = _pack(out[0:16, :])

    def step_light(t, first):
        lay = 0 if first else 1
        if ostream and not first:
            ocopy(t - 4).start()
        mold = memh32[...]
        tok = xn32[seg_rows32(t), :] if first else hn32[seg_rows32(t - 1), :]
        h = _unpack(jnp.concatenate([mold, tok], axis=0))
        upd_l1(t - 1)
        upd_l2(t - 3)
        if first:
            ln_next(t)
        outs = attn_block(h, fill2_ref[lay], 2 * M + SEG, lagqk_l, lagpv_l)
        out = jnp.concatenate(outs, axis=1)
        out_s[seg_rows(lay), :] = out[16:, :]
        if first:
            rowl = lax.broadcasted_iota(jnp.int32, (M, D), 0) >> 2
            memh32[...] = jnp.where(rowl == 0, _pack(out[0:16, :]), mold)
        else:
            memh32[...] = _pack(out[0:16, :])

    lax.fori_loop(0, 2, lambda t, c: (step_light(t, True), c)[1], 0)
    lax.fori_loop(2, 2 + nfull, lambda t, c: (step_full(t), c)[1], 0, unroll=unroll)
    lax.fori_loop(NSEG, NSEG + 2, lambda t, c: (step_light(t, False), c)[1], 0)
    upd_l2(NSEG - 1)
    if ostream:
        ocopy(NSEG - 2).start()
        ocopy(NSEG - 1).start()
        pltpu.make_async_copy(o_s, o_ref, sems.at[0]).wait()


def make(**kw):
    Fm, G2, fill, fill2 = _consts()

    @jax.jit
    def run(A_x, A_mem0, A_Wq, A_Wk, A_Wv, A_Wo, B_k, B_v, B_shift_k, B_ssm_k, B_ssm_D):
        hbm = pl.BlockSpec(memory_space=pltpu.HBM)
        vm = pl.BlockSpec()
        wr = lambda w: w.reshape(D // 16, 8, 2, H, DH)
        out = pl.pallas_call(
            functools.partial(kernel, **kw),
            out_shape=jax.ShapeDtypeStruct((S, D), BF16),
            out_specs=hbm if kw.get('ostream', True) else vm,
            in_specs=[hbm, vm, hbm, hbm, hbm, hbm, hbm, hbm, vm, hbm, vm, vm, vm, vm, vm],
            scratch_shapes=[
                pltpu.VMEM((S, D) if kw.get('ospos', 0) == 1 else (8, 128), BF16),
                pltpu.VMEM((S, D), BF16),
                pltpu.VMEM((S, D), BF16),
                pltpu.VMEM((S, D), BF16),
                pltpu.VMEM((D, S), BF16),
                pltpu.VMEM((3, D // 16, 8, 2, H, DH), BF16),
                pltpu.VMEM((H * DH, D), BF16),
                pltpu.VMEM((H, 3, D // 2, DH), U32),
                pltpu.VMEM((NCT, H * DH // 2, 128), U32),
                pltpu.VMEM((NCT, NCH, 2 * C, 128), F32),
                pltpu.VMEM((NCT, NCH, 2 * C, 128), F32),
                pltpu.VMEM((S, D), F32),
                pltpu.VMEM((S // 2 + SEG // 2, D), U32),
                pltpu.VMEM((S + 2 * SEG, D), F32),
                pltpu.VMEM((S // 2 + SEG, D), U32),
                pltpu.VMEM((2 * SEG, D), F32),
                pltpu.VMEM((M, D), U32),
                pltpu.VMEM((R // 2, H * DH), U32),
                pltpu.VMEM((S, D) if (kw.get('ospos', 0) == 0 and kw.get('ostream', True)) else (8, 128), BF16),
                pltpu.SemaphoreType.DMA((16,)),
            ],
            compiler_params=pltpu.CompilerParams(vmem_limit_bytes=120 * 1024 * 1024),
        )(A_x.reshape(S, D), A_mem0.reshape(M, D), wr(A_Wq), wr(A_Wk), wr(A_Wv), A_Wo.reshape(H * DH, D),
          B_k.reshape(S, D), B_v.reshape(S, D), B_shift_k.T, B_ssm_k, B_ssm_D.reshape(1, D),
          jnp.asarray(Fm), jnp.asarray(G2), jnp.asarray(fill), jnp.asarray(fill2))
        return out.reshape(1, S, D)
    return run


_RUN = make()


def pallas_interleave_layers__memory_aug_recurrent_mem_tr__ssm_conv_h3__prompt_kernel(
        A_x, A_mem0, A_Wq, A_Wk, A_Wv, A_Wo, A_seg_len, B_q, B_k, B_v, B_shift_k, B_ssm_k, B_ssm_D):
    assert int(A_seg_len) == SEG and A_x.shape == (1, S, D) and A_Wq.shape == (D, H, DH)
    del B_q
    return _RUN(A_x, A_mem0, A_Wq, A_Wk, A_Wv, A_Wo, B_k, B_v, B_shift_k, B_ssm_k, B_ssm_D)
```

```python
import numpy as np
import jax
import jax.numpy as jnp
from jax import lax
from jax.experimental import pallas as pl
from jax.experimental.pallas import tpu as pltpu

S, D, H, DH, M, SEG = 2048, 640, 32, 128, 8, 32
NSEG = S // SEG
R2 = 2 * (M + SEG)
R1 = M + SEG
C = 128
NCH = S // C
NCT = D // 128
NDB = D // 16
F32, BF16, U32 = jnp.float32, jnp.bfloat16, jnp.uint32
EPS = 1e-5
SCALE = DH ** -0.5
NSPL = 4
XP = 256


def _consts():
    import ml_dtypes
    f = np.arange(C)[:, None].astype(np.float64)
    t = np.arange(C)[None, :].astype(np.float64)
    th = np.pi * (2 * f + 1) * t / (2 * C)
    fwd = np.concatenate([np.cos(th), -np.sin(th)], 0)
    inv = np.concatenate([np.cos(th.T), -np.sin(th.T)], 1) / C
    fill2 = np.full((R2, 128), -np.inf, np.float32)
    layer = lambda i: 0 if (i < M or 2 * M <= i < 2 * M + SEG) else 1
    for i in range(R2):
        for j in range(R2):
            if layer(i) == layer(j):
                keep = i < 2 * M or j < 2 * M or (i - 2 * M) % SEG >= (j - 2 * M) % SEG
                fill2[i, j] = 0.0 if keep else -1e9
    fill1 = np.full((R1, 128), -np.inf, np.float32)
    for i in range(R1):
        for j in range(R1):
            fill1[i, j] = 0.0 if (i < M or i >= j) else -1e9
    to_bf16 = lambda a: a.astype(np.float32).astype(ml_dtypes.bfloat16)
    return to_bf16(fwd), to_bf16(inv), fill2, fill1


def _ln(x):
    xc = x - jnp.mean(x, axis=-1, keepdims=True)
    return xc * lax.rsqrt(jnp.mean(xc * xc, axis=-1, keepdims=True) + EPS)


def _pack(x):
    return pltpu.bitcast(x.astype(BF16), U32)


def _unpack(x):
    return pltpu.bitcast(x, BF16)


def _rows(s, n):
    return pl.ds(pl.multiple_of(s * n, n), n)


def _kernel(x_hbm, mem0_hbm, wq_hbm, wk_hbm, wv_hbm, wo_hbm, bk_hbm, bv_hbm, sh_hbm, ssmk_hbm, ssmd_hbm,
            fwd_hbm, inv_hbm, fill2_hbm, fill1_hbm,
            o_hbm,
            mem0_s, sh_s, ssmd_s, fwd_s, inv_s, fill2_s, fill1_s,
            x_s, bk_s, bv_s, ssmk_s, raw_s, woraw_s, w32, wo32,
            kpad_s, u_s, kf_s, y_s, xn32, x2_s, hn32, out_s, mem32, a32, af32, o_s, sems):
    order = []

    def cpy(src, dst):
        order.append(pltpu.make_async_copy(src, dst, sems.at[1 + len(order)]))
        return order[-1]
    PR = S // NSPL
    c_b0 = [cpy(sh_hbm, sh_s), cpy(ssmd_hbm, ssmd_s), cpy(fwd_hbm, fwd_s)]
    c_ssmk = cpy(ssmk_hbm, ssmk_s)
    c_kv = [(cpy(bk_hbm.at[pl.ds(i * PR, PR)], bk_s.at[pl.ds(i * PR, PR)]),
             cpy(bv_hbm.at[pl.ds(i * PR, PR)], bv_s.at[pl.ds(i * PR, PR)])) for i in range(NSPL)]
    c_x0 = cpy(x_hbm.at[pl.ds(0, XP)], x_s.at[pl.ds(0, XP)])
    c_a0 = [cpy(mem0_hbm, mem0_s), cpy(inv_hbm, inv_s), cpy(fill2_hbm, fill2_s), cpy(fill1_hbm, fill1_s)]
    c_w = [cpy(wq_hbm, raw_s.at[0]), cpy(wk_hbm, raw_s.at[1]), cpy(wv_hbm, raw_s.at[2]), cpy(wo_hbm, woraw_s)]
    c_x1 = cpy(x_hbm.at[pl.ds(XP, S - XP)], x_s.at[pl.ds(XP, S - XP)])
    for c_ in order:
        c_.start()

    out_s[...] = jnp.zeros_like(out_s)
    x2_s[0:SEG, :] = jnp.zeros((SEG, D), F32)
    hn32[0:SEG // 2, :] = jnp.zeros((SEG // 2, D), U32)
    for c in range(NCT):
        kpad_s[c, 0:8, :] = jnp.zeros((8, 128), F32)

    for c_ in c_b0:
        c_.wait()
    sh = sh_s[...].astype(F32)
    dd = ssmd_s[...].astype(F32)
    fwd = fwd_s[...]
    c_ssmk.wait()
    for a in range(NCH):
        for c in range(NCT):
            kf_s[c, a] = lax.dot_general(fwd, ssmk_s[c * 128:(c + 1) * 128, a * C:(a + 1) * C],
                                         (((1,), (1,)), ((), ())), preferred_element_type=F32)
    for a in range(NCH):
        r0 = a * C
        if r0 % PR == 0:
            c_kv[r0 // PR][0].wait()
            c_kv[r0 // PR][1].wait()
        for c in range(NCT):
            cs = slice(c * 128, (c + 1) * 128)
            cur = bk_s[r0:r0 + C, cs].astype(F32)
            kpad_s[c, r0 + 8:r0 + 8 + C, :] = cur
            ks = cur * sh[0:1, cs]
            for m in range(1, 4):
                ks = ks + kpad_s[c, r0 + 8 - m:r0 + 8 - m + C, :] * sh[m:m + 1, cs]
            kv = (ks * bv_s[r0:r0 + C, cs].astype(F32)).astype(BF16)
            y_s[r0:r0 + C, cs] = kv.astype(F32) * dd[:, cs]
            u_s[c, a] = jnp.dot(fwd, kv, preferred_element_type=F32)

    c_x0.wait()
    for c_ in c_a0:
        c_.wait()
    xn32[0:SEG // 2, :] = _pack(_ln(x_s[0:SEG, :].astype(F32)))
    mem0f = mem0_s[...].astype(F32)
    mem32[...] = _pack(jnp.concatenate([mem0f, mem0f], axis=0))

    sgn = jnp.where((lax.broadcasted_iota(jnp.int32, (8, 128), 0) & 1) == 0, 1.0, -1.0).astype(F32)

    def cmac(i, carry):
        c = i // 16
        re = pl.ds(pl.multiple_of((i % 16) * 8, 8), 8)
        im = pl.ds(pl.multiple_of((i % 16) * 8 + C, 8), 8)
        ur = [u_s[c, a, re, :] for a in range(NCH)]
        ui = [u_s[c, a, im, :] for a in range(NCH)]
        for a in range(NCH):
            yr = yi = None
            for j in range(a + 1):
                kr, ki = kf_s[c, j, re, :], kf_s[c, j, im, :]
                tr = kr * ur[a - j] - ki * ui[a - j]
                ti = kr * ui[a - j] + ki * ur[a - j]
                yr, yi = (tr, ti) if yr is None else (yr + tr, yi + ti)
            zr, zi = (yr, yi) if a == 0 else (yr - sgn * pyi, yi + sgn * pyr)
            pyr, pyi = yr, yi
            u_s[c, a, re, :] = zr
            u_s[c, a, im, :] = zi
        return carry
    lax.fori_loop(0, NCT * 16, cmac, 0, unroll=2)

    def wblock(part, db):
        r0 = pl.multiple_of(db * 8, 8)
        e = pltpu.bitcast(raw_s[part, db, :, 0], U32)
        o = pltpu.bitcast(raw_s[part, db, :, 1], U32)
        lo = jnp.transpose((e & 0xFFFF) | (o << 16), (1, 0, 2))
        hi = jnp.transpose((e >> 16) | (o & np.uint32(0xFFFF0000)), (1, 0, 2))
        for hp in range(H // 2):
            w32[2 * hp, part, pl.ds(r0, 8), :] = lo[hp]
            w32[2 * hp + 1, part, pl.ds(r0, 8), :] = hi[hp]

    invm = inv_s[...]

    def inv_and_wqk(a, carry):
        r0 = pl.multiple_of(a * C, C)
        for c in range(NCT):
            y_s[pl.ds(r0, C), c * 128:(c + 1) * 128] += jnp.dot(invm, u_s[c, a].astype(BF16),
                                                                preferred_element_type=F32)
            wblock(a >> 3, (a & 7) * 5 + c)
        return carry
    c_w[0].wait()
    lax.fori_loop(0, 8, inv_and_wqk, 0, unroll=4)
    c_w[1].wait()
    lax.fori_loop(8, NCH, inv_and_wqk, 0, unroll=4)
    c_w[2].wait()
    lax.fori_loop(0, NDB, lambda db, c_: (wblock(2, db), c_)[1], 0, unroll=2)
    c_w[3].wait()

    def wo_block(hd, carry):
        for j in range(NCT):
            wo32[j, _rows(hd, DH // 2), :] = pltpu.bitcast(woraw_s[_rows(hd, DH), j * 128:(j + 1) * 128], U32)
        return carry
    lax.fori_loop(0, H, wo_block, 0)

    def upd_l1(s1):
        sc = jnp.clip(s1, 0, NSEG - 1)
        x1 = x_s[_rows(sc, SEG), :].astype(F32) + out_s[0:SEG, :]
        x2 = x1 + _ln(x1) * y_s[_rows(sc, SEG), :]
        x2_s[_rows(s1 + 1, SEG), :] = x2
        hn32[_rows(s1 + 1, SEG // 2), :] = _pack(_ln(x2))

    def upd_l2(s2):
        sc = jnp.clip(s2, 0, NSEG - 1)
        x3 = x2_s[_rows(jnp.clip(s2 + 1, 0, NSEG), SEG), :] + out_s[SEG:2 * SEG, :]
        o_s[_rows(sc, SEG), :] = (x3 + _ln(x3) * y_s[_rows(sc, SEG), :]).astype(BF16)

    def ln_next(t):
        xn32[_rows(jnp.minimum(t + 1, NSEG), SEG // 2), :] = _pack(
            _ln(x_s[_rows(jnp.minimum(t + 1, NSEG - 1), SEG), :].astype(F32)))

    def ocopy(u):
        return pltpu.make_async_copy(o_s.at[_rows(u, SEG)], o_hbm.at[_rows(u, SEG)], sems.at[0])

    def attn(h, fill, lagqk, lagpv):
        nrow = h.shape[0]
        lhs_f32 = h.dtype == F32
        zpad = jnp.zeros((128 - nrow, DH), F32)
        lhs = (lambda v_: v_.astype(BF16).astype(F32)) if lhs_f32 else (lambda v_: v_.astype(BF16))
        rhs = lambda v_: jnp.concatenate([v_, zpad], axis=0).astype(BF16)
        proj = lambda hd, part: jnp.dot(h, _unpack(w32[hd, part]), preferred_element_type=F32)
        qs, ks, vs, ps, ls, acc = {}, {}, {}, {}, {}, {}
        done = [0] * NCT

        def qk(i):
            s_ = lax.dot_general(qs.pop(i), ks.pop(i), (((1,), (1,)), ((), ())), preferred_element_type=F32)
            s_ = jnp.where(fill < 0, fill, s_ * SCALE)
            e = jnp.exp(s_ - jnp.max(s_, axis=-1, keepdims=True))
            l = jnp.sum(e, axis=-1, keepdims=True)
            r = pl.reciprocal(l, approx=True)
            ls[i] = r * (2.0 - l * r)
            ps[i] = lhs(e)

        def pv(i):
            a_ = jnp.dot(ps.pop(i), vs.pop(i), preferred_element_type=F32) * ls.pop(i)
            if lhs_f32:
                af32[:, i * DH:(i + 1) * DH] = lhs(a_)
            else:
                a32[:, i * DH:(i + 1) * DH] = _pack(a_)

        def oproj(j, h0, h1):
            a_ = af32[:, h0 * DH:h1 * DH] if lhs_f32 else _unpack(a32[:, h0 * DH:h1 * DH])
            r = jnp.dot(a_, _unpack(wo32[j, h0 * (DH // 2):h1 * (DH // 2), :]), preferred_element_type=F32)
            acc[j] = r if j not in acc else acc[j] + r
            done[j] = h1

        def oproj_fill(n, ready):
            for j in range(NCT):
                k_ = min(n, ready - done[j])
                if k_ > 0:
                    oproj(j, done[j], done[j] + k_)
                    n -= k_
        for hd in range(H + lagpv):
            ready = max(hd - lagpv - 2, 0)
            if hd < H:
                ks[hd] = rhs(proj(hd, 1))
            else:
                oproj_fill(5, ready)
            if 0 <= hd - lagqk < H:
                qk(hd - lagqk)
            if hd < H:
                qs[hd] = lhs(proj(hd, 0))
                vs[hd] = rhs(proj(hd, 2))
            else:
                oproj_fill(10, ready)
            if 0 <= hd - lagpv < H:
                pv(hd - lagpv)
        oproj_fill(28, H - 2)
        for j in range(NCT):
            if done[j] < H:
                oproj(j, done[j], H)
        return jnp.concatenate([acc[j] for j in range(NCT)], axis=1)

    def step_two(t, carry):
        @pl.when(t >= 4)
        def _():
            ocopy(t - 4).start()
        h = _unpack(jnp.concatenate([mem32[...], xn32[_rows(t, SEG // 2), :],
                                     hn32[_rows(t - 1, SEG // 2), :]], axis=0))
        upd_l1(t - 1)
        upd_l2(t - 3)
        ln_next(t)
        out = attn(h, fill2_s[...], 1, 2)
        out_s[...] = out[2 * M:, :]
        mem32[...] = _pack(out[0:2 * M, :])
        return carry

    def step_one(t, first):
        lay = 0 if first else 1
        if not first:
            ocopy(t - 4).start()
        mold = _unpack(mem32[...]).astype(F32)
        tok = xn32[_rows(t, SEG // 2), :] if first else hn32[_rows(t - 1, SEG // 2), :]
        h = jnp.concatenate([mold[M * lay:M * lay + M], _unpack(tok).astype(F32)], axis=0)
        upd_l1(t - 1)
        upd_l2(t - 3)
        if first:
            ln_next(t)
        out = attn(h, fill1_s[...], 2, 4)
        out_s[lay * SEG:(lay + 1) * SEG, :] = out[M:, :]
        mnew = [out[0:M], mold[M:]] if first else [mold[0:M], out[0:M]]
        mem32[...] = _pack(jnp.concatenate(mnew, axis=0))

    lax.fori_loop(0, 2, lambda t, c_: (step_one(t, True), c_)[1], 0)
    c_x1.wait()
    lax.fori_loop(2, NSEG, step_two, 0, unroll=2)
    lax.fori_loop(NSEG, NSEG + 2, lambda t, c_: (step_one(t, False), c_)[1], 0)
    ocopy(NSEG - 2).start()
    upd_l2(NSEG - 1)
    ocopy(NSEG - 1).start()
    pltpu.make_async_copy(o_s, o_hbm, sems.at[0]).wait()


@jax.jit
def _run(A_x, A_mem0, A_Wq, A_Wk, A_Wv, A_Wo, B_k, B_v, B_shift_k, B_ssm_k, B_ssm_D):
    fwd, inv, fill2, fill1 = _consts()
    wr = lambda w: w.reshape(NDB, 8, 2, H, DH)
    out = pl.pallas_call(
        _kernel,
        out_shape=jax.ShapeDtypeStruct((S, D), BF16),
        in_specs=[pl.BlockSpec(memory_space=pltpu.HBM)] * 15,
        out_specs=pl.BlockSpec(memory_space=pltpu.HBM),
        scratch_shapes=[
            pltpu.VMEM((M, D), BF16),
            pltpu.VMEM((4, D), BF16),
            pltpu.VMEM((1, D), BF16),
            pltpu.VMEM((2 * C, C), BF16),
            pltpu.VMEM((C, 2 * C), BF16),
            pltpu.VMEM((R2, 128), F32),
            pltpu.VMEM((R1, 128), F32),
            pltpu.VMEM((S, D), BF16),
            pltpu.VMEM((S, D), BF16),
            pltpu.VMEM((S, D), BF16),
            pltpu.VMEM((D, S), BF16),
            pltpu.VMEM((3, NDB, 8, 2, H, DH), BF16),
            pltpu.VMEM((H * DH, D), BF16),
            pltpu.VMEM((H, 3, D // 2, DH), U32),
            pltpu.VMEM((NCT, H * DH // 2, 128), U32),
            pltpu.VMEM((NCT, S + 8, 128), F32),
            pltpu.VMEM((NCT, NCH, 2 * C, 128), F32),
            pltpu.VMEM((NCT, NCH, 2 * C, 128), F32),
            pltpu.VMEM((S, D), F32),
            pltpu.VMEM((S // 2 + SEG // 2, D), U32),
            pltpu.VMEM((S + 2 * SEG, D), F32),
            pltpu.VMEM((S // 2 + SEG, D), U32),
            pltpu.VMEM((2 * SEG, D), F32),
            pltpu.VMEM((M, D), U32),
            pltpu.VMEM((R2 // 2, H * DH), U32),
            pltpu.VMEM((R1, H * DH), F32),
            pltpu.VMEM((S, D), BF16),
            pltpu.SemaphoreType.DMA((24,)),
        ],
        compiler_params=pltpu.CompilerParams(vmem_limit_bytes=112 * 1024 * 1024),
    )(A_x.reshape(S, D), A_mem0.reshape(M, D), wr(A_Wq), wr(A_Wk), wr(A_Wv), A_Wo.reshape(H * DH, D),
      B_k.reshape(S, D), B_v.reshape(S, D), B_shift_k.T, B_ssm_k, B_ssm_D.reshape(1, D),
      jnp.asarray(fwd), jnp.asarray(inv), jnp.asarray(fill2), jnp.asarray(fill1))
    return out.reshape(1, S, D)


def pallas_interleave_layers__memory_aug_recurrent_mem_tr__ssm_conv_h3__prompt_kernel(
        A_x, A_mem0, A_Wq, A_Wk, A_Wv, A_Wo, A_seg_len, B_q, B_k, B_v, B_shift_k, B_ssm_k, B_ssm_D):
    assert int(A_seg_len) == SEG and A_x.shape == (1, S, D) and A_Wq.shape == (D, H, DH)
    assert A_mem0.shape == (1, M, D) and B_shift_k.shape == (D, 4) and B_ssm_k.shape == (D, S)
    del B_q
    return _run(A_x, A_mem0, A_Wq, A_Wk, A_Wv, A_Wo, B_k, B_v, B_shift_k, B_ssm_k, B_ssm_D)
```

```python
import numpy as np
import jax
import jax.numpy as jnp
from jax import lax
from jax.experimental import pallas as pl
from jax.experimental.pallas import tpu as pltpu

S, D, H, DH, M, SEG = 2048, 640, 32, 128, 8, 32
NSEG = S // SEG
R2 = 2 * (M + SEG)
R1 = M + SEG
C = 128
NCH = S // C
NCT = D // 128
NDB = D // 16
F32, BF16, U32 = jnp.float32, jnp.bfloat16, jnp.uint32
EPS = 1e-5
SCALE = DH ** -0.5
NSPL = 4
XP = 256


def _consts():
    import ml_dtypes
    f = np.arange(C)[:, None].astype(np.float64)
    t = np.arange(C)[None, :].astype(np.float64)
    th = np.pi * (2 * f + 1) * t / (2 * C)
    fwd = np.concatenate([np.cos(th), -np.sin(th)], 0)
    inv = np.concatenate([np.cos(th.T), -np.sin(th.T)], 1) / C
    fill2 = np.full((R2, 128), -np.inf, np.float32)
    layer = lambda i: 0 if (i < M or 2 * M <= i < 2 * M + SEG) else 1
    for i in range(R2):
        for j in range(R2):
            if layer(i) == layer(j):
                keep = i < 2 * M or j < 2 * M or (i - 2 * M) % SEG >= (j - 2 * M) % SEG
                fill2[i, j] = 0.0 if keep else -1e9
    fill1 = np.full((R1, 128), -np.inf, np.float32)
    for i in range(R1):
        for j in range(R1):
            fill1[i, j] = 0.0 if (i < M or i >= j) else -1e9
    to_bf16 = lambda a: a.astype(np.float32).astype(ml_dtypes.bfloat16)
    return to_bf16(fwd), to_bf16(inv), fill2, fill1


def _ln(x):
    xc = x - jnp.mean(x, axis=-1, keepdims=True)
    return xc * lax.rsqrt(jnp.mean(xc * xc, axis=-1, keepdims=True) + EPS)


def _pack(x):
    return pltpu.bitcast(x.astype(BF16), U32)


def _unpack(x):
    return pltpu.bitcast(x, BF16)


def _rows(s, n):
    return pl.ds(pl.multiple_of(s * n, n), n)


def _kernel(x_hbm, mem0_hbm, wq_hbm, wk_hbm, wv_hbm, wo_hbm, bk_hbm, bv_hbm, sh_hbm, ssmk_hbm, ssmd_hbm,
            fwd_hbm, inv_hbm, fill2_hbm, fill1_hbm,
            o_hbm,
            mem0_s, sh_s, ssmd_s, fwd_s, inv_s, fill2_s, fill1_s,
            x_s, bk_s, bv_s, ssmk_s, raw_s, woraw_s, w32, wo32,
            kpad_s, u_s, kf_s, y_s, xn32, x2_s, hn32, out_s, mem32, a32, af32, o_s, sems):
    order = []

    def cpy(src, dst):
        order.append(pltpu.make_async_copy(src, dst, sems.at[1 + len(order)]))
        return order[-1]
    PR = S // NSPL
    c_b0 = [cpy(sh_hbm, sh_s), cpy(ssmd_hbm, ssmd_s), cpy(fwd_hbm, fwd_s)]
    c_ssmk = cpy(ssmk_hbm, ssmk_s)
    c_kv = [(cpy(bk_hbm.at[pl.ds(i * PR, PR)], bk_s.at[pl.ds(i * PR, PR)]),
             cpy(bv_hbm.at[pl.ds(i * PR, PR)], bv_s.at[pl.ds(i * PR, PR)])) for i in range(NSPL)]
    c_x0 = cpy(x_hbm.at[pl.ds(0, XP)], x_s.at[pl.ds(0, XP)])
    c_a0 = [cpy(mem0_hbm, mem0_s), cpy(inv_hbm, inv_s), cpy(fill2_hbm, fill2_s), cpy(fill1_hbm, fill1_s)]
    c_w = [cpy(wq_hbm, raw_s.at[0]), cpy(wk_hbm, raw_s.at[1]), cpy(wv_hbm, raw_s.at[2]), cpy(wo_hbm, woraw_s)]
    c_x1 = cpy(x_hbm.at[pl.ds(XP, S - XP)], x_s.at[pl.ds(XP, S - XP)])
    for c_ in order:
        c_.start()

    out_s[...] = jnp.zeros_like(out_s)
    x2_s[0:SEG, :] = jnp.zeros((SEG, D), F32)
    hn32[0:SEG // 2, :] = jnp.zeros((SEG // 2, D), U32)
    for c in range(NCT):
        kpad_s[c, 0:8, :] = jnp.zeros((8, 128), F32)

    for c_ in c_b0:
        c_.wait()
    sh = sh_s[...].astype(F32)
    dd = ssmd_s[...].reshape(1, D).astype(F32)
    fwd = fwd_s[...]
    c_ssmk.wait()
    for a in range(NCH):
        for c in range(NCT):
            kf_s[c, a] = lax.dot_general(fwd, ssmk_s[c * 128:(c + 1) * 128, a * C:(a + 1) * C],
                                         (((1,), (1,)), ((), ())), preferred_element_type=F32)
    for a in range(NCH):
        r0 = a * C
        if r0 % PR == 0:
            c_kv[r0 // PR][0].wait()
            c_kv[r0 // PR][1].wait()
        for c in range(NCT):
            cs = slice(c * 128, (c + 1) * 128)
            cur = bk_s[r0:r0 + C, cs].astype(F32)
            kpad_s[c, r0 + 8:r0 + 8 + C, :] = cur
            ks = cur * sh[0:1, cs]
            for m in range(1, 4):
                ks = ks + kpad_s[c, r0 + 8 - m:r0 + 8 - m + C, :] * sh[m:m + 1, cs]
            kv = (ks * bv_s[r0:r0 + C, cs].astype(F32)).astype(BF16)
            y_s[r0:r0 + C, cs] = kv.astype(F32) * dd[:, cs]
            u_s[c, a] = jnp.dot(fwd, kv, preferred_element_type=F32)

    c_x0.wait()
    for c_ in c_a0:
        c_.wait()
    xn32[0:SEG // 2, :] = _pack(_ln(x_s[0:SEG, :].astype(F32)))
    mem0f = mem0_s[...].astype(F32)
    mem32[...] = _pack(jnp.concatenate([mem0f, mem0f], axis=0))

    sgn = jnp.where((lax.broadcasted_iota(jnp.int32, (8, 128), 0) & 1) == 0, 1.0, -1.0).astype(F32)

    def cmac(i, carry):
        c = i // 16
        re = pl.ds(pl.multiple_of((i % 16) * 8, 8), 8)
        im = pl.ds(pl.multiple_of((i % 16) * 8 + C, 8), 8)
        ur = [u_s[c, a, re, :] for a in range(NCH)]
        ui = [u_s[c, a, im, :] for a in range(NCH)]
        for a in range(NCH):
            yr = yi = None
            for j in range(a + 1):
                kr, ki = kf_s[c, j, re, :], kf_s[c, j, im, :]
                tr = kr * ur[a - j] - ki * ui[a - j]
                ti = kr * ui[a - j] + ki * ur[a - j]
                yr, yi = (tr, ti) if yr is None else (yr + tr, yi + ti)
            zr, zi = (yr, yi) if a == 0 else (yr - sgn * pyi, yi + sgn * pyr)
            pyr, pyi = yr, yi
            u_s[c, a, re, :] = zr
            u_s[c, a, im, :] = zi
        return carry
    lax.fori_loop(0, NCT * 16, cmac, 0, unroll=4)

    def wblock(part, db):
        r0 = pl.multiple_of(db * 8, 8)
        e = pltpu.bitcast(raw_s[part, db, :, 0], U32)
        o = pltpu.bitcast(raw_s[part, db, :, 1], U32)
        lo = jnp.transpose((e & 0xFFFF) | (o << 16), (1, 0, 2))
        hi = jnp.transpose((e >> 16) | (o & np.uint32(0xFFFF0000)), (1, 0, 2))
        for hp in range(H // 2):
            w32[2 * hp, part, pl.ds(r0, 8), :] = lo[hp]
            w32[2 * hp + 1, part, pl.ds(r0, 8), :] = hi[hp]

    invm = inv_s[...]

    def inv_and_wqk(a, carry):
        r0 = pl.multiple_of(a * C, C)
        for c in range(NCT):
            y_s[pl.ds(r0, C), c * 128:(c + 1) * 128] += jnp.dot(invm, u_s[c, a].astype(BF16),
                                                                preferred_element_type=F32)
            wblock(a >> 3, (a & 7) * 5 + c)
        return carry
    c_w[0].wait()
    lax.fori_loop(0, 8, inv_and_wqk, 0, unroll=True)
    c_w[1].wait()
    lax.fori_loop(8, NCH, inv_and_wqk, 0, unroll=True)
    c_w[2].wait()
    lax.fori_loop(0, NDB, lambda db, c_: (wblock(2, db), c_)[1], 0, unroll=4)
    c_w[3].wait()

    def wo_block(hd, carry):
        for j in range(NCT):
            wo32[j, _rows(hd, DH // 2), :] = pltpu.bitcast(woraw_s[_rows(hd, DH), j * 128:(j + 1) * 128], U32)
        return carry
    lax.fori_loop(0, H, wo_block, 0)

    def upd_l1(s1):
        sc = jnp.clip(s1, 0, NSEG - 1)
        x1 = x_s[_rows(sc, SEG), :].astype(F32) + out_s[0:SEG, :]
        x2 = x1 + _ln(x1) * y_s[_rows(sc, SEG), :]
        x2_s[_rows(s1 + 1, SEG), :] = x2
        hn32[_rows(s1 + 1, SEG // 2), :] = _pack(_ln(x2))

    def upd_l2(s2):
        sc = jnp.clip(s2, 0, NSEG - 1)
        x3 = x2_s[_rows(jnp.clip(s2 + 1, 0, NSEG), SEG), :] + out_s[SEG:2 * SEG, :]
        o_s[_rows(sc, SEG), :] = (x3 + _ln(x3) * y_s[_rows(sc, SEG), :]).astype(BF16)

    def ln_next(t):
        xn32[_rows(jnp.minimum(t + 1, NSEG), SEG // 2), :] = _pack(
            _ln(x_s[_rows(jnp.minimum(t + 1, NSEG - 1), SEG), :].astype(F32)))

    def ocopy(u):
        return pltpu.make_async_copy(o_s.at[_rows(u, SEG)], o_hbm.at[_rows(u, SEG)], sems.at[0])

    def attn(h, fill, lagqk, lagpv):
        nrow = h.shape[0]
        lhs_f32 = h.dtype == F32
        zpad = jnp.zeros((128 - nrow, DH), F32)
        lhs = (lambda v_: v_.astype(BF16).astype(F32)) if lhs_f32 else (lambda v_: v_.astype(BF16))
        rhs = lambda v_: jnp.concatenate([v_, zpad], axis=0).astype(BF16)
        proj = lambda hd, part: jnp.dot(h, _unpack(w32[hd, part]), preferred_element_type=F32)
        qs, ks, vs, ps, ls, acc = {}, {}, {}, {}, {}, {}
        done = [0] * NCT

        def qk(i):
            s_ = lax.dot_general(qs.pop(i), ks.pop(i), (((1,), (1,)), ((), ())), preferred_element_type=F32)
            s_ = jnp.where(fill < 0, fill, s_ * SCALE)
            e = jnp.exp(s_ - jnp.max(s_, axis=-1, keepdims=True))
            l = jnp.sum(e, axis=-1, keepdims=True)
            r = pl.reciprocal(l, approx=True)
            ls[i] = r * (2.0 - l * r)
            ps[i] = lhs(e)

        def pv(i):
            a_ = jnp.dot(ps.pop(i), vs.pop(i), preferred_element_type=F32) * ls.pop(i)
            if lhs_f32:
                af32[:, i * DH:(i + 1) * DH] = lhs(a_)
            else:
                a32[:, i * DH:(i + 1) * DH] = _pack(a_)

        def oproj(j, h0, h1):
            a_ = af32[:, h0 * DH:h1 * DH] if lhs_f32 else _unpack(a32[:, h0 * DH:h1 * DH])
            r = jnp.dot(a_, _unpack(wo32[j, h0 * (DH // 2):h1 * (DH // 2), :]), preferred_element_type=F32)
            acc[j] = r if j not in acc else acc[j] + r
            done[j] = h1

        def oproj_fill(n, ready):
            for j in range(NCT):
                k_ = min(n, ready - done[j])
                if k_ > 0:
                    oproj(j, done[j], done[j] + k_)
                    n -= k_
        for hd in range(H + lagpv):
            ready = max(hd - lagpv - 2, 0)
            if hd < H:
                ks[hd] = rhs(proj(hd, 1))
            else:
                oproj_fill(5, ready)
            if 0 <= hd - lagqk < H:
                qk(hd - lagqk)
            if hd < H:
                qs[hd] = lhs(proj(hd, 0))
                vs[hd] = rhs(proj(hd, 2))
            else:
                oproj_fill(10, ready)
            if 0 <= hd - lagpv < H:
                pv(hd - lagpv)
        oproj_fill(28, H - 2)
        for j in range(NCT):
            if done[j] < H:
                oproj(j, done[j], H)
        return jnp.concatenate([acc[j] for j in range(NCT)], axis=1)

    def step_two(t, carry):
        @pl.when(t >= 4)
        def _():
            ocopy(t - 4).start()
        h = _unpack(jnp.concatenate([mem32[...], xn32[_rows(t, SEG // 2), :],
                                     hn32[_rows(t - 1, SEG // 2), :]], axis=0))
        upd_l1(t - 1)
        upd_l2(t - 3)
        ln_next(t)
        out = attn(h, fill2_s[...], 1, 2)
        out_s[...] = out[2 * M:, :]
        mem32[...] = _pack(out[0:2 * M, :])
        return carry

    def step_one(t, first):
        lay = 0 if first else 1
        if not first:
            ocopy(t - 4).start()
        mold = _unpack(mem32[...]).astype(F32)
        tok = xn32[_rows(t, SEG // 2), :] if first else hn32[_rows(t - 1, SEG // 2), :]
        h = jnp.concatenate([mold[M * lay:M * lay + M], _unpack(tok).astype(F32)], axis=0)
        upd_l1(t - 1)
        upd_l2(t - 3)
        if first:
            ln_next(t)
        out = attn(h, fill1_s[...], 2, 4)
        out_s[lay * SEG:(lay + 1) * SEG, :] = out[M:, :]
        mnew = [out[0:M], mold[M:]] if first else [mold[0:M], out[0:M]]
        mem32[...] = _pack(jnp.concatenate(mnew, axis=0))

    lax.fori_loop(0, 2, lambda t, c_: (step_one(t, True), c_)[1], 0)
    c_x1.wait()
    lax.fori_loop(2, NSEG, step_two, 0, unroll=2)
    lax.fori_loop(NSEG, NSEG + 2, lambda t, c_: (step_one(t, False), c_)[1], 0)
    ocopy(NSEG - 2).start()
    upd_l2(NSEG - 1)
    ocopy(NSEG - 1).start()
    pltpu.make_async_copy(o_s, o_hbm, sems.at[0]).wait()


@jax.jit
def _run(A_x, A_mem0, A_Wq, A_Wk, A_Wv, A_Wo, B_k, B_v, B_shift_k, B_ssm_k, B_ssm_D):
    fwd, inv, fill2, fill1 = _consts()
    wr = lambda w: w.reshape(NDB, 8, 2, H, DH)
    out = pl.pallas_call(
        _kernel,
        out_shape=jax.ShapeDtypeStruct((S, D), BF16),
        in_specs=[pl.BlockSpec(memory_space=pltpu.HBM)] * 15,
        out_specs=pl.BlockSpec(memory_space=pltpu.HBM),
        scratch_shapes=[
            pltpu.VMEM((M, D), BF16),
            pltpu.VMEM((4, D), BF16),
            pltpu.VMEM((D,), BF16),
            pltpu.VMEM((2 * C, C), BF16),
            pltpu.VMEM((C, 2 * C), BF16),
            pltpu.VMEM((R2, 128), F32),
            pltpu.VMEM((R1, 128), F32),
            pltpu.VMEM((S, D), BF16),
            pltpu.VMEM((S, D), BF16),
            pltpu.VMEM((S, D), BF16),
            pltpu.VMEM((D, S), BF16),
            pltpu.VMEM((3, NDB, 8, 2, H, DH), BF16),
            pltpu.VMEM((H * DH, D), BF16),
            pltpu.VMEM((H, 3, D // 2, DH), U32),
            pltpu.VMEM((NCT, H * DH // 2, 128), U32),
            pltpu.VMEM((NCT, S + 8, 128), F32),
            pltpu.VMEM((NCT, NCH, 2 * C, 128), F32),
            pltpu.VMEM((NCT, NCH, 2 * C, 128), F32),
            pltpu.VMEM((S, D), F32),
            pltpu.VMEM((S // 2 + SEG // 2, D), U32),
            pltpu.VMEM((S + 2 * SEG, D), F32),
            pltpu.VMEM((S // 2 + SEG, D), U32),
            pltpu.VMEM((2 * SEG, D), F32),
            pltpu.VMEM((M, D), U32),
            pltpu.VMEM((R2 // 2, H * DH), U32),
            pltpu.VMEM((R1, H * DH), F32),
            pltpu.VMEM((S, D), BF16),
            pltpu.SemaphoreType.DMA((24,)),
        ],
        compiler_params=pltpu.CompilerParams(vmem_limit_bytes=112 * 1024 * 1024),
    )(A_x.reshape(S, D), A_mem0.reshape(M, D), wr(A_Wq), wr(A_Wk), wr(A_Wv), A_Wo.reshape(H * DH, D),
      B_k.reshape(S, D), B_v.reshape(S, D), B_shift_k.T, B_ssm_k, B_ssm_D,
      jnp.asarray(fwd), jnp.asarray(inv), jnp.asarray(fill2), jnp.asarray(fill1))
    return out.reshape(1, S, D)


def pallas_interleave_layers__memory_aug_recurrent_mem_tr__ssm_conv_h3__prompt_kernel(
        A_x, A_mem0, A_Wq, A_Wk, A_Wv, A_Wo, A_seg_len, B_q, B_k, B_v, B_shift_k, B_ssm_k, B_ssm_D):
    assert int(A_seg_len) == SEG and A_x.shape == (1, S, D) and A_Wq.shape == (D, H, DH)
    assert A_mem0.shape == (1, M, D) and B_shift_k.shape == (D, 4) and B_ssm_k.shape == (D, S)
    del B_q
    return _run(A_x, A_mem0, A_Wq, A_Wk, A_Wv, A_Wo, B_k, B_v, B_shift_k, B_ssm_k, B_ssm_D)
```
